```python
import os as _os
_os.environ.setdefault("JAX_PLATFORMS", "cpu")
import jax
import jax.numpy as jnp

def _softmax(x, axis=-1):
    return jax.nn.softmax(x, axis=axis)
def _gelu(x):
    return jax.nn.gelu(x, approximate=True)
def _silu(x):
    return jax.nn.silu(x)
def _sigmoid(x):
    return jax.nn.sigmoid(x)
def _layernorm(x, axis=-1, eps=1e-5):
    m = jnp.mean(x, axis=axis, keepdims=True)
    v = jnp.var(x, axis=axis, keepdims=True)
    return (x - m) / jnp.sqrt(v + eps)
def _scatter_add(tgt, idx, src, axis=0):
    return tgt.at[idx].add(src)
def _segment_sum(src, seg, n):
    return jax.ops.segment_sum(src, seg, n)
class _Rng:
    def __init__(self, key):
        self._k = key
    def _next(self):
        self._k, sub = jax.random.split(self._k)
        return sub
    def normal(self, shape):
        return jax.random.normal(self._next(), shape, dtype=jnp.bfloat16)
    def randint(self, lo, hi, shape):
        return jax.random.randint(self._next(), shape, lo, hi, dtype=jnp.int32)
    def uniform(self, shape, lo=0.0, hi=1.0):
        return jax.random.uniform(self._next(), shape, jnp.bfloat16, lo, hi)
    def permutation(self, n):
        return jax.random.permutation(self._next(), n)


kernel_name = 'gated_mix__linear_attn_block__swiglu_ffn__prompt'

def setup_inputs():
    _rng = _Rng(jax.random.key(int.from_bytes(__import__("os").urandom(4), "little")))
    _w = (lambda a: (lambda t: t.astype(jnp.bfloat16) if jnp.issubdtype(t.dtype, jnp.floating) else t)(jnp.asarray(a)))
    def _A_setup():
        B, S, D = 1, 2048, 512
        return {
            "x": _w((lambda *s: _rng.normal(s) * 0.05)(B, S, D)),
            "wqkv": _w((lambda *s: _rng.normal(s) * 0.8)(D, 3 * D)),
            "wo": _w((lambda *s: _rng.normal(s) * 0.05)(D, D)),
        }
    _A_in = _A_setup()

    def _B_setup():
        B, S, D, F = 1, 2048, 512, 1792
        return {
            "x": _w((lambda *s: _rng.normal(s) * 0.05)(B, S, D)),
            "w_gate": _w((lambda *s: _rng.normal(s) * 0.1)(D, F)),
            "w_up": _w((lambda *s: _rng.normal(s) * 0.1)(D, F)),
            "w_down": _w((lambda *s: _rng.normal(s) * 0.1)(F, D)),
        }
    _B_in = _B_setup()

    return {
        "A_x": _A_in["x"],
        "A_wqkv": _A_in["wqkv"],
        "A_wo": _A_in["wo"],
        "B_x": _B_in["x"],
        "B_w_gate": _B_in["w_gate"],
        "B_w_up": _B_in["w_up"],
        "B_w_down": _B_in["w_down"],
        "gate_w": _w((lambda *s: _rng.normal(s) * 0.05)(512) * 16.0),
    }

def reference(A_x, A_wqkv, A_wo, B_x, B_w_gate, B_w_up, B_w_down, gate_w):
    def _A_ref(x, wqkv, wo):
        B, S, D = x.shape
        H = 32; Dh = D // H
        qkv = (lambda x, *d: x.transpose(*d))((x @ wqkv).reshape(B, S, 3, H, Dh), 2, 0, 3, 1, 4)
        q, k, v = qkv[0], qkv[1], qkv[2]
        phi = lambda t: jnp.where(t > 0, t + 1, jnp.exp(t)) + 1e-6
        pq, pk = phi(q), phi(k)
        kv = jnp.einsum("bhsd,bhse->bhde", pk, v)
        z = jnp.einsum("bhsd->bhd", pk)
        num = jnp.einsum("bhqd,bhde->bhqe", pq, kv)
        den = jnp.einsum("bhqd,bhd->bhq", pq, z)[..., None] + 1e-6
        o = num / den
        return (lambda x, *d: x.transpose(*d))(o, 0, 2, 1, 3).reshape(B, S, D) @ wo

    def _B_ref(x, w_gate, w_up, w_down):
        g = _silu(x @ w_gate)
        u = x @ w_up
        return (g * u) @ w_down

    x = A_x
    g = _sigmoid((x * gate_w).sum(-1, keepdims=True))
    a = _A_ref(x, A_wqkv, A_wo)
    b = _B_ref(x, B_w_gate, B_w_up, B_w_down)
    return g * a + (1 - g) * b
```

```python
import functools
import jax
import jax.numpy as jnp
from jax import lax
import jax.experimental.pallas as pl
import jax.experimental.pallas.tpu as pltpu

S, D, F = 2048, 512, 1792
H, DH = 32, 16
BF = jnp.bfloat16
F32 = jnp.float32
L = 128
HD = D // 2
HS = S // 2


def _phi(t):
    return jnp.where(t > 0, t + 1.0, jnp.exp(t)) + 1e-6


def _dot(a, b):
    return jnp.dot(a, b, preferred_element_type=F32)


def _dot_nt(a, b):
    return lax.dot_general(a, b, (((1,), (1,)), ((), ())), preferred_element_type=F32)


def _scope(name, on):
    import contextlib
    return jax.named_scope(name) if on else contextlib.nullcontext()


def _swap_lane_bit(a, b, k):
    lane = lax.broadcasted_iota(jnp.int32, a.shape, 1)
    lo = (lane & k) == 0
    return (jnp.where(lo, a, pltpu.roll(b, k, 1)),
            jnp.where(lo, pltpu.roll(a, L - k, 1), b))


def _perm_lanes(blocks):
    b0, b1, b2, b3 = blocks
    b0, b2 = _swap_lane_bit(b0, b2, 8)
    b1, b3 = _swap_lane_bit(b1, b3, 8)
    b0, b1 = _swap_lane_bit(b0, b1, 4)
    b2, b3 = _swap_lane_bit(b2, b3, 4)
    return [b0, b1, b2, b3]


def _lhs7(a11, a12, a21, a22):
    return [(a11 + a22).astype(BF), (a21 + a22).astype(BF), a11.astype(BF), a22.astype(BF),
            (a11 + a12).astype(BF), (a21 - a11).astype(BF), (a12 - a22).astype(BF)]


def _rhs7f(f11, f12, f21, f22):
    return [(f11 + f22).astype(BF), f11.astype(BF), (f12 - f22).astype(BF), (f21 - f11).astype(BF),
            f22.astype(BF), (f11 + f12).astype(BF), (f21 + f22).astype(BF)]


def _rhs7(b11, b12, b21, b22):
    r = _rhs7f(*[b.astype(F32) for b in (b11, b12, b21, b22)])
    r[1] = b11
    r[4] = b22
    return r


def _pk(v):
    return pltpu.bitcast(v, jnp.uint32)


def _upk(v):
    return pltpu.bitcast(v, BF)


def _comb(m):
    return (m[0] + m[3] - m[4] + m[6], m[2] + m[4], m[1] + m[3], m[0] - m[1] + m[2] + m[5])


_R_AS_L = (0, 2, 6, 5, 3, 4, 1)
_SUMS = (0, 1, 4, 5, 6)


def _kernel(x_hbm, wqkv_hbm, wo_hbm, wg_hbm, wu_hbm, wd_hbm, gw_hbm, out_hbm,
            x_v, wqkv_v, wo_v, wg_v, wu_v, wd_v, gw_v, rk_v, wq_v, lx_v, p_acc, z_acc, m_v, zr_v,
            pq_v, g_v, o_buf, sem, *, XS, KT, QT, HM, FC, OC, ORD1, AQ, SC):
    X0, X1 = XS

    def cp(src, dst, k):
        return pltpu.make_async_copy(src, dst, sem.at[k])

    def xcp(a, b, k):
        return cp(x_hbm.at[:, pl.ds(a, b - a), :], x_v.at[:, pl.ds(a, b - a), :], k)

    def wcp(c0, n, k):
        return cp(wqkv_hbm.at[:, pl.ds(c0, n)], wqkv_v.at[:, pl.ds(c0, n)], k)

    g1 = [wcp(D, HD, 0)]
    g2 = [wcp(D + HD, HD, 1)]
    g3 = [cp(gw_hbm, gw_v, 2), xcp(0, X0, 2)]
    g4 = [xcp(X0, X1, 0)]
    g5 = [xcp(X1, HS, 1), wcp(0, D, 1), wcp(2 * D, D, 1), cp(wo_hbm, wo_v, 1)]
    g6 = [cp(wg_hbm, wg_v, 2), cp(wu_hbm, wu_v, 2), cp(wd_hbm, wd_v, 2)]

    def start(g):
        for c in g:
            c.start()

    def wait(g, name):
        with _scope(name, SC):
            for c in g:
                c.wait()

    def lx(i, r0, n):
        return _upk(lx_v[i, pl.ds(r0 // 2, n // 2), :])

    def kpath(a, b):
        rows = slice(a, b)
        n = b - a
        xa = x_v[0, rows, :].astype(F32)
        xb = x_v[1, rows, :].astype(F32)
        l7 = _lhs7(xa[:, :HD], xa[:, HD:], xb[:, :HD], xb[:, HD:])
        l7[2] = x_v[0, rows, :HD]
        l7[3] = x_v[1, rows, HD:]
        for i in range(7):
            lx_v[i, a // 2:b // 2, :] = _pk(l7[i])
        gw = gw_v[...].astype(F32).reshape(1, D)
        for k, xf in enumerate((xa, xb)):
            gl = jnp.sum(xf * gw, axis=1, keepdims=True)
            g_v[k, rows, :] = jnp.broadcast_to(0.5 * jnp.tanh(0.5 * gl), (n, L))
        m = [None] * 7
        for i in (3, 1, 2, 4, 0, 6, 5):
            m[i] = _dot_nt(_upk(rk_v[i]), l7[i])
        c11, c12, c21, c22 = [_phi(c) for c in _comb(m)]
        for k, (u, v) in enumerate(((c11, c21), (c12, c22))):
            w = u + v
            zs = w[:, 0:L]
            for j in range(1, n // L):
                zs = zs + w[:, j * L:(j + 1) * L]
            if a == 0:
                z_acc[k * HD:(k + 1) * HD, :] = zs
            else:
                z_acc[k * HD:(k + 1) * HD, :] += zs
        lp = _lhs7(c11, c21, c12, c22)
        for i in (2, 4, 5, 3, 0, 1, 6):
            p = _dot(lp[i], l7[_R_AS_L[i]])
            if a == 0:
                p_acc[i] = p
            else:
                p_acc[i] += p

    def krange(a, e):
        while a < e:
            b = min(a + KT, e)
            kpath(a, b)
            a = b

    start(g1)
    start(g2)
    start(g3)
    wait(g1, "w1")
    start(g4)
    ta = wqkv_v[:, D:D + HD].astype(F32).T
    rk_v[1] = _pk(ta[:, :HD].astype(BF))
    rk_v[3] = _pk((ta[:, HD:] - ta[:, :HD]).astype(BF))
    rk_v[6] = _pk(ta[:, HD:].astype(BF))
    wait(g2, "w2")
    start(g5)
    tb = wqkv_v[:, D + HD:2 * D].astype(F32).T
    b11 = _upk(rk_v[1]).astype(F32)
    rk_v[0] = _pk((b11 + tb[:, HD:]).astype(BF))
    rk_v[2] = _pk((tb[:, :HD] - tb[:, HD:]).astype(BF))
    rk_v[4] = _pk(tb[:, HD:].astype(BF))
    rk_v[5] = _pk((b11 + tb[:, :HD]).astype(BF))
    rk_v[6] = _pk((_upk(rk_v[6]).astype(F32) + tb[:, HD:]).astype(BF))
    wait(g3, "w3")
    start(g6)
    krange(0, X0)
    wait(g4, "w4")
    krange(X0, X1)
    wait(g5, "w5")
    blocks = [pltpu.bitcast(wqkv_v[:, j * L:(j + 1) * L], jnp.uint32) for j in range(4)]
    blocks = _perm_lanes(blocks)
    wq = jnp.concatenate([pltpu.bitcast(blk, BF) for blk in blocks], axis=1)
    for i, r in enumerate(_rhs7(wq[:HD, :HD], wq[:HD, HD:], wq[HD:, :HD], wq[HD:, HD:])):
        wq_v[i] = _pk(r)
    krange(X1, HS)

    def qproj(t):
        rows = slice(t * QT, (t + 1) * QT)
        m = [None] * 7
        for i in ORD1:
            m[i] = _dot(lx(i, t * QT, QT), _upk(wq_v[i]))
        c11, c12, c21, c22 = _comb(m)
        pq_v[0, rows, :HD] = _phi(c11)
        pq_v[0, rows, HD:] = _phi(c12)
        pq_v[1, rows, :HD] = _phi(c21)
        pq_v[1, rows, HD:] = _phi(c22)

    zrow = jnp.sum(z_acc[...].T, axis=0, keepdims=True)
    zb = _perm_lanes([jnp.broadcast_to(zrow[:, j * L:(j + 1) * L], (8, L)) for j in range(4)])
    for j in range(4):
        zr_v[:, j * L:(j + 1) * L] = zb[j]

    qproj(0)
    p11, p12, p21, p22 = _comb([p_acc[i] for i in range(7)])
    pp = jnp.concatenate([jnp.concatenate([p11, p12], axis=1), jnp.concatenate([p21, p22], axis=1)], axis=0).astype(BF)
    row = lax.broadcasted_iota(jnp.int32, (L, L), 0) // DH
    col = lax.broadcasted_iota(jnp.int32, (L, L), 1) // DH
    same = row == col
    mb = []
    for b in range(D // L):
        sl = slice(b * L, (b + 1) * L)
        kv = _dot(pp[sl, :], wqkv_v[:, 2 * D + b * L: 2 * D + (b + 1) * L])
        kv = jnp.where(same, kv, 0.0).astype(BF)
        mb.append(_dot(kv, wo_v[sl, :]).reshape(16, 8, D))
    sub_lo = lax.broadcasted_iota(jnp.int32, (16, 8, D), 1) < 4
    xs = []
    for b1 in range(2):
        a_, b_ = mb[2 * b1], mb[2 * b1 + 1]
        xs.append((jnp.where(sub_lo, a_, pltpu.roll(b_, 4, 1)).reshape(8, 2, 8, D),
                   jnp.where(sub_lo, pltpu.roll(a_, 4, 1), b_).reshape(8, 2, 8, D)))
    mh = []
    for d3 in range(2):
        mh.append(jnp.concatenate(
            [jnp.concatenate([xs[0][d2][:, d3], xs[1][d2][:, d3]], axis=1).reshape(L, D) for d2 in range(2)], axis=0))
    for i, r in enumerate(_rhs7f(mh[0][:, :HD], mh[0][:, HD:], mh[1][:, :HD], mh[1][:, HD:])):
        m_v[i] = _pk(r)
    for t in range(1, HS // QT):
        qproj(t)

    wait(g6, "w6")

    def o_start(k, r0, nr, c0, nc):
        cp(o_buf.at[k, pl.ds(r0, nr), pl.ds(c0, nc)], out_hbm.at[k, pl.ds(r0, nr), pl.ds(c0, nc)], 0).start()

    def qnorm(k, rows, n):
        pq = pq_v[k, rows, :]
        r = pq * zr_v[0:1, :]
        s = (r[:, 0:L] + r[:, L:2 * L]) + (r[:, 2 * L:3 * L] + r[:, 3 * L:4 * L])
        lane = lax.broadcasted_iota(jnp.int32, (n, L), 1)
        s = s + jnp.where((lane & 1) == 0, pltpu.roll(s, L - 1, 1), pltpu.roll(s, 1, 1))
        s = s + jnp.where((lane & 2) == 0, pltpu.roll(s, L - 2, 1), pltpu.roll(s, 2, 1))
        scale = (0.5 + g_v[k, rows, :]) / (s + 1e-6)
        return jnp.concatenate([pq[:, j * L:(j + 1) * L] * scale for j in range(4)], axis=1)

    def ffn(t, carry):
        r0 = pl.multiple_of(t * HM, HM)
        rows = pl.ds(r0, HM)
        rp = pl.multiple_of(t * (HM // 2), HM // 2)
        HF = FC // 2
        nch = F // FC
        ha = jnp.concatenate([0.25 - 0.5 * g_v[0, rows, :]] * (HF // L), axis=1)
        hb = jnp.concatenate([0.25 - 0.5 * g_v[1, rows, :]] * (HF // L), axis=1)

        def act(gu, hs):
            g = gu[:, :HF]
            return (g * hs) * (1.0 + jnp.tanh(0.5 * g)) * gu[:, HF:]

        lh = [[] for _ in range(7)]
        rd = [[] for _ in range(7)]
        aq = [[] for _ in range(7)]
        QR = HM // len(AQ)

        def attn(j):
            rj = pl.ds(pl.multiple_of(r0 + j * QR, QR), QR)
            qa = qnorm(0, rj, QR)
            qb = qnorm(1, rj, QR)
            lq = _lhs7(qa[:, :HD], qa[:, HD:], qb[:, :HD], qb[:, HD:])
            for i in range(7):
                aq[i].append(_dot(lq[i], _upk(m_v[i])))

        for c in range(nch):
            k1 = slice(c * FC, c * FC + HF)
            k2 = slice(c * FC + HF, (c + 1) * FC)
            rg = _rhs7(wg_v[:HD, k1], wg_v[:HD, k2], wg_v[HD:, k1], wg_v[HD:, k2])
            ru = _rhs7(wu_v[:HD, k1], wu_v[:HD, k2], wu_v[HD:, k1], wu_v[HD:, k2])
            rw = [jnp.concatenate([p, q], axis=1) for p, q in zip(rg, ru)]
            m = [None] * 7
            for n_, i in enumerate(ORD1):
                if (c, n_) in AQ:
                    attn(AQ.index((c, n_)))
                m[i] = _dot(_upk(lx_v[i, pl.ds(rp, HM // 2), :]), rw[i])
            c11, c12, c21, c22 = _comb(m)
            l7 = _lhs7(act(c11, ha), act(c12, ha), act(c21, hb), act(c22, hb))
            r7 = _rhs7(wd_v[k1, :HD], wd_v[k1, HD:], wd_v[k2, :HD], wd_v[k2, HD:])
            for i in range(7):
                lh[i].append(l7[i])
                rd[i].append(r7[i])

        aq = [jnp.concatenate(v, axis=0) for v in aq]

        def down(i, c0=0, c1=nch, ks=slice(None)):
            return _dot(jnp.concatenate([v[ks, :] for v in lh[i][c0:c1]], axis=1), jnp.concatenate(rd[i][c0:c1], axis=0))

        def emit(k, rk, c0, val):
            nr, nc = val.shape
            o_buf[k, pl.ds(rk, nr), c0:c0 + nc] = val.astype(BF)
            o_start(k, rk, nr, c0, nc)

        m3 = (aq[2] + down(2, 0, nch - 1)) + down(2, nch - 1, nch)
        m5 = aq[4] + down(4)
        emit(0, r0, HD, m3 + m5)
        m2 = aq[1] + down(1)
        m4 = aq[3] + down(3)
        emit(1, r0, 0, m2 + m4)
        m1 = aq[0] + down(0)
        m7 = aq[6] + down(6)
        emit(0, r0, 0, m1 + m4 - m5 + m7)
        part = m1 - m2 + m3 + aq[5]
        k0 = 0
        for k, nr in enumerate(OC):
            ks = slice(k0, k0 + nr)
            res = part[ks, :] + down(5, ks=ks)
            rk = pl.multiple_of(r0 + k0, L)
            if k < len(OC) - 1:
                emit(1, rk, HD, res)
            else:
                emit(1, rk, HD, res[:, :L])
                emit(1, rk, HD + L, res[:, L:])
            k0 += nr
        return carry

    with _scope("ffn", SC):
        lax.fori_loop(0, HS // HM, ffn, 0)
    with _scope("waito", SC):
        cp(o_buf, out_hbm, 0).wait()


def impl(A_x, A_wqkv, A_wo, B_x, B_w_gate, B_w_up, B_w_down, gate_w,
         XS=(128, 640), KT=256, QT=256, HM=512, FC=256, OC=(256, 128, 128), ORD1=(2, 4, 1, 3, 0, 6, 5), AQ=((1, 4), (2, 4), (3, 4), (4, 4)),
         SC=False):
    x = A_x.reshape(2, HS, D)
    any_spec = pl.BlockSpec(memory_space=pl.ANY)
    out = pl.pallas_call(
        functools.partial(_kernel, XS=XS, KT=KT, QT=QT, HM=HM, FC=FC, OC=OC, ORD1=ORD1, AQ=AQ, SC=SC),
        out_shape=jax.ShapeDtypeStruct((2, HS, D), BF),
        in_specs=[any_spec] * 7,
        out_specs=any_spec,
        scratch_shapes=[
            pltpu.VMEM((2, HS, D), BF),
            pltpu.VMEM((D, 3 * D), BF),
            pltpu.VMEM((D, D), BF),
            pltpu.VMEM((D, F), BF),
            pltpu.VMEM((D, F), BF),
            pltpu.VMEM((F, D), BF),
            pltpu.VMEM((D,), BF),
            pltpu.VMEM((7, HD // 2, HD), jnp.uint32),
            pltpu.VMEM((7, HD // 2, HD), jnp.uint32),
            pltpu.VMEM((7, HS // 2, HD), jnp.uint32),
            pltpu.VMEM((7, HD, HD), F32),
            pltpu.VMEM((D, L), F32),
            pltpu.VMEM((7, HD // 2, HD), jnp.uint32),
            pltpu.VMEM((8, D), F32),
            pltpu.VMEM((2, HS, D), F32),
            pltpu.VMEM((2, HS, L), F32),
            pltpu.VMEM((2, HS, D), BF),
            pltpu.SemaphoreType.DMA((3,)),
        ],
        compiler_params=pltpu.CompilerParams(vmem_limit_bytes=100 * 1024 * 1024, disable_bounds_checks=True,
                                             disable_semaphore_checks=True),
    )(x, A_wqkv, A_wo, B_w_gate, B_w_up, B_w_down, gate_w)
    return out.reshape(1, S, D)


@jax.jit
def pallas_gated_mix__linear_attn_block__swiglu_ffn__prompt_kernel(A_x, A_wqkv, A_wo, B_x, B_w_gate, B_w_up, B_w_down, gate_w):
    return impl(A_x, A_wqkv, A_wo, B_x, B_w_gate, B_w_up, B_w_down, gate_w)
```

```python
import functools
import jax
import jax.numpy as jnp
from jax import lax
import jax.experimental.pallas as pl
import jax.experimental.pallas.tpu as pltpu

S, D, F = 2048, 512, 1792
H, DH = 32, 16
BF = jnp.bfloat16
F32 = jnp.float32
L = 128
HD = D // 2
HS = S // 2


def _phi(t):
    return jnp.where(t > 0, t + 1.0, jnp.exp(t)) + 1e-6


def _dot(a, b):
    return jnp.dot(a, b, preferred_element_type=F32)


def _dot_nt(a, b):
    return lax.dot_general(a, b, (((1,), (1,)), ((), ())), preferred_element_type=F32)


def _scope(name, on):
    import contextlib
    return jax.named_scope(name) if on else contextlib.nullcontext()


def _swap_lane_bit(a, b, k):
    lane = lax.broadcasted_iota(jnp.int32, a.shape, 1)
    lo = (lane & k) == 0
    return (jnp.where(lo, a, pltpu.roll(b, k, 1)),
            jnp.where(lo, pltpu.roll(a, L - k, 1), b))


def _perm_lanes(blocks):
    b0, b1, b2, b3 = blocks
    b0, b2 = _swap_lane_bit(b0, b2, 8)
    b1, b3 = _swap_lane_bit(b1, b3, 8)
    b0, b1 = _swap_lane_bit(b0, b1, 4)
    b2, b3 = _swap_lane_bit(b2, b3, 4)
    return [b0, b1, b2, b3]


def _lhs7(a11, a12, a21, a22):
    return [(a11 + a22).astype(BF), (a21 + a22).astype(BF), a11.astype(BF), a22.astype(BF),
            (a11 + a12).astype(BF), (a21 - a11).astype(BF), (a12 - a22).astype(BF)]


def _rhs7f(f11, f12, f21, f22):
    return [(f11 + f22).astype(BF), f11.astype(BF), (f12 - f22).astype(BF), (f21 - f11).astype(BF),
            f22.astype(BF), (f11 + f12).astype(BF), (f21 + f22).astype(BF)]


def _rhs7(b11, b12, b21, b22):
    r = _rhs7f(*[b.astype(F32) for b in (b11, b12, b21, b22)])
    r[1] = b11
    r[4] = b22
    return r


def _l7f(a11, a12, a21, a22):
    return [a11 + a22, a21 + a22, a11, a22, a11 + a12, a21 - a11, a12 - a22]


def _r7f(f11, f12, f21, f22):
    return [f11 + f22, f11, f12 - f22, f21 - f11, f22, f11 + f12, f21 + f22]


_LT = (((1, 0), (1, 3)), ((1, 2), (1, 3)), ((1, 0),), ((1, 3),), ((1, 0), (1, 1)), ((1, 2), (-1, 0)), ((1, 1), (-1, 3)))
_RT = (((1, 0), (1, 3)), ((1, 0),), ((1, 1), (-1, 3)), ((1, 2), (-1, 0)), ((1, 3),), ((1, 0), (1, 1)), ((1, 2), (1, 3)))


def _term(terms, get):
    v = get(terms[0][1])
    for sg, q in terms[1:]:
        v = v + get(q) if sg > 0 else v - get(q)
    return v


def _quads(v):
    r, c = v.shape[0] // 2, v.shape[1] // 2
    return v[:r, :c], v[:r, c:], v[r:, :c], v[r:, c:]


def _pk(v):
    return pltpu.bitcast(v, jnp.uint32)


def _upk(v):
    return pltpu.bitcast(v, BF)


def _comb(m):
    return (m[0] + m[3] - m[4] + m[6], m[2] + m[4], m[1] + m[3], m[0] - m[1] + m[2] + m[5])


KAPPA = 16.0
KAPPA_OUT = 4.0


def _sub(v):
    n, c = v.shape
    return v.reshape(n // 32, 4, 8, c)[:, 0].reshape(n // 4, c)


def _colmax(v):
    return jnp.max(jnp.abs(v), axis=0, keepdims=True)


def _col_growth(m1, c11, c22, dbg=False):
    t = jnp.minimum(jnp.sum(jnp.abs(c11), axis=0, keepdims=True), jnp.sum(jnp.abs(c22), axis=0, keepdims=True))
    if dbg:
        return _colmax(m1) / t * c11.shape[0]
    return _colmax(m1) - (KAPPA / c11.shape[0]) * t


def _lanefold(v, op):
    r = v[:, 0:L]
    for j in range(1, v.shape[1] // L):
        r = op(r, v[:, j * L:(j + 1) * L])
    return r


_R_AS_L = (0, 2, 6, 5, 3, 4, 1)
_SUMS = (0, 1, 4, 5, 6)


def _kernel(x_hbm, wqkv_hbm, wo_hbm, wg_hbm, wu_hbm, wd_hbm, gw_hbm, out_hbm,
            x_v, wqkv_v, wo_v, wg_v, wu_v, wd_v, gw_v, rk_v, wq_v, lx_v, p_acc, z_acc, m_v, h_v, acc_v, mo_v, zr_v,
            pq_v, g_v, ks_v, chk_v, fa_v, fz_v, o_buf, sem, *, GUARD, DBG, XS, KT, QT, HM, FC, OC, ORD1, L2SET, FIRST, SCHED, SC):
    X0, X1 = XS

    def cp(src, dst, k):
        return pltpu.make_async_copy(src, dst, sem.at[k])

    def xcp(a, b, k):
        return cp(x_hbm.at[:, pl.ds(a, b - a), :], x_v.at[:, pl.ds(a, b - a), :], k)

    def wcp(c0, n, k):
        return cp(wqkv_hbm.at[:, pl.ds(c0, n)], wqkv_v.at[:, pl.ds(c0, n)], k)

    g1 = [wcp(D, HD, 0)]
    g2 = [wcp(D + HD, HD, 1)]
    g3 = [cp(gw_hbm, gw_v, 2), xcp(0, X0, 2)]
    g4 = [xcp(X0, X1, 0)]
    g5 = [xcp(X1, HS, 1), wcp(0, D, 1), wcp(2 * D, D, 1), cp(wo_hbm, wo_v, 1)]
    g6 = [cp(wg_hbm, wg_v, 2), cp(wu_hbm, wu_v, 2), cp(wd_hbm, wd_v, 2)]

    def start(g):
        for c in g:
            c.start()

    def wait(g, name):
        with _scope(name, SC):
            for c in g:
                c.wait()

    def lx(i, r0, n):
        return _upk(lx_v[i, pl.ds(r0 // 2, n // 2), :])

    def kpath(a, b):
        rows = slice(a, b)
        n = b - a
        xa = x_v[0, rows, :].astype(F32)
        xb = x_v[1, rows, :].astype(F32)
        l7 = _lhs7(xa[:, :HD], xa[:, HD:], xb[:, :HD], xb[:, HD:])
        l7[2] = x_v[0, rows, :HD]
        l7[3] = x_v[1, rows, HD:]
        for i in range(7):
            lx_v[i, a // 2:b // 2, :] = _pk(l7[i])
        gw = gw_v[...].astype(F32).reshape(1, D)
        for k, xf in enumerate((xa, xb)):
            gl = jnp.sum(xf * gw, axis=1, keepdims=True)
            g_v[k, rows, :] = jnp.broadcast_to(0.5 * jnp.tanh(0.5 * gl), (n, L))
        m = [None] * 7
        for i in (3, 1, 2, 4, 0, 6, 5):
            m[i] = _dot_nt(_upk(rk_v[i]), l7[i])
        kq = _comb(m)
        if GUARD:
            st = (_lanefold(jnp.abs(m[0]), jnp.maximum), _lanefold(jnp.abs(kq[0]), jnp.add), _lanefold(jnp.abs(kq[3]), jnp.add))
            if a == 0:
                for k in range(3):
                    ks_v[k] = st[k]
            else:
                ks_v[0] = jnp.maximum(ks_v[0], st[0])
                ks_v[1] += st[1]
                ks_v[2] += st[2]
        c11, c12, c21, c22 = [_phi(c) for c in kq]
        for k, (u, v) in enumerate(((c11, c21), (c12, c22))):
            w = u + v
            zs = w[:, 0:L]
            for j in range(1, n // L):
                zs = zs + w[:, j * L:(j + 1) * L]
            if a == 0:
                z_acc[k * HD:(k + 1) * HD, :] = zs
            else:
                z_acc[k * HD:(k + 1) * HD, :] += zs
        lp = _lhs7(c11, c21, c12, c22)
        for i in (2, 4, 5, 3, 0, 1, 6):
            p = _dot(lp[i], l7[_R_AS_L[i]])
            if a == 0:
                p_acc[i] = p
            else:
                p_acc[i] += p

    def krange(a, e):
        while a < e:
            b = min(a + KT, e)
            kpath(a, b)
            a = b

    start(g1)
    start(g2)
    start(g3)
    wait(g1, "w1")
    start(g4)
    ta = wqkv_v[:, D:D + HD].astype(F32).T
    rk_v[1] = _pk(ta[:, :HD].astype(BF))
    rk_v[3] = _pk((ta[:, HD:] - ta[:, :HD]).astype(BF))
    rk_v[6] = _pk(ta[:, HD:].astype(BF))
    wait(g2, "w2")
    start(g5)
    tb = wqkv_v[:, D + HD:2 * D].astype(F32).T
    b11 = _upk(rk_v[1]).astype(F32)
    rk_v[0] = _pk((b11 + tb[:, HD:]).astype(BF))
    rk_v[2] = _pk((tb[:, :HD] - tb[:, HD:]).astype(BF))
    rk_v[4] = _pk(tb[:, HD:].astype(BF))
    rk_v[5] = _pk((b11 + tb[:, :HD]).astype(BF))
    rk_v[6] = _pk((_upk(rk_v[6]).astype(F32) + tb[:, HD:]).astype(BF))
    wait(g3, "w3")
    start(g6)
    krange(0, X0)
    wait(g4, "w4")
    krange(X0, X1)
    wait(g5, "w5")
    blocks = [pltpu.bitcast(wqkv_v[:, j * L:(j + 1) * L], jnp.uint32) for j in range(4)]
    blocks = _perm_lanes(blocks)
    wq = jnp.concatenate([pltpu.bitcast(blk, BF) for blk in blocks], axis=1)
    for i, r in enumerate(_rhs7(wq[:HD, :HD], wq[:HD, HD:], wq[HD:, :HD], wq[HD:, HD:])):
        wq_v[i] = _pk(r)
    krange(X1, HS)

    viol = {"q": []}

    def qproj(t):
        rows = slice(t * QT, (t + 1) * QT)
        m = [None] * 7
        for i in ORD1:
            m[i] = _dot(lx(i, t * QT, QT), _upk(wq_v[i]))
        c11, c12, c21, c22 = _comb(m)
        if GUARD:
            viol["q"].append(_col_growth(m[0], _sub(c11) if QT >= 512 else c11[::1], _sub(c22) if QT >= 512 else c22[::1], DBG))
        pq_v[0, rows, :HD] = _phi(c11)
        pq_v[0, rows, HD:] = _phi(c12)
        pq_v[1, rows, :HD] = _phi(c21)
        pq_v[1, rows, HD:] = _phi(c22)

    zrow = jnp.sum(z_acc[...].T, axis=0, keepdims=True)
    zb = _perm_lanes([jnp.broadcast_to(zrow[:, j * L:(j + 1) * L], (8, L)) for j in range(4)])
    for j in range(4):
        zr_v[:, j * L:(j + 1) * L] = zb[j]

    qproj(0)
    p11, p12, p21, p22 = _comb([p_acc[i] for i in range(7)])
    pp = jnp.concatenate([jnp.concatenate([p11, p12], axis=1), jnp.concatenate([p21, p22], axis=1)], axis=0).astype(BF)
    row = lax.broadcasted_iota(jnp.int32, (L, L), 0) // DH
    col = lax.broadcasted_iota(jnp.int32, (L, L), 1) // DH
    same = row == col
    mb = []
    for b in range(D // L):
        sl = slice(b * L, (b + 1) * L)
        kv = _dot(pp[sl, :], wqkv_v[:, 2 * D + b * L: 2 * D + (b + 1) * L])
        kv = jnp.where(same, kv, 0.0).astype(BF)
        mb.append(_dot(kv, wo_v[sl, :]).reshape(16, 8, D))
    sub_lo = lax.broadcasted_iota(jnp.int32, (16, 8, D), 1) < 4
    xs = []
    for b1 in range(2):
        a_, b_ = mb[2 * b1], mb[2 * b1 + 1]
        xs.append((jnp.where(sub_lo, a_, pltpu.roll(b_, 4, 1)).reshape(8, 2, 8, D),
                   jnp.where(sub_lo, pltpu.roll(a_, 4, 1), b_).reshape(8, 2, 8, D)))
    mh = []
    for d3 in range(2):
        mh.append(jnp.concatenate(
            [jnp.concatenate([xs[0][d2][:, d3], xs[1][d2][:, d3]], axis=1).reshape(L, D) for d2 in range(2)], axis=0))
    m_v[:HD, :] = mh[0]
    m_v[HD:, :] = mh[1]
    for t in range(1, HS // QT):
        qproj(t)
    if GUARD:
        pm = p_acc[0]
        chk_v[0:1, :] = functools.reduce(jnp.maximum, viol["q"])
        chk_v[1:2, :] = _col_growth(pm, p11, p22, DBG)
        chk_v[2:3, :] = _col_growth(pm.T, p11.T, p22.T, DBG)
        kt = jnp.minimum(jnp.sum(ks_v[1].T, axis=0, keepdims=True), jnp.sum(ks_v[2].T, axis=0, keepdims=True))
        kg = jnp.max(ks_v[0].T, axis=0, keepdims=True)
        chk_v[3:4, :] = kg / kt * HS if DBG else kg - (KAPPA / HS) * kt
        chk_v[4:8, :] = jnp.zeros((4, HD), F32)

    wait(g6, "w6")

    def o_start(k, r0, nr, c0, nc):
        cp(o_buf.at[k, pl.ds(r0, nr), pl.ds(c0, nc)], out_hbm.at[k, pl.ds(r0, nr), pl.ds(c0, nc)], 0).start()

    def qnorm(k, rows, n):
        pq = pq_v[k, rows, :]
        r = pq * zr_v[0:1, :]
        s = (r[:, 0:L] + r[:, L:2 * L]) + (r[:, 2 * L:3 * L] + r[:, 3 * L:4 * L])
        lane = lax.broadcasted_iota(jnp.int32, (n, L), 1)
        s = s + jnp.where((lane & 1) == 0, pltpu.roll(s, L - 1, 1), pltpu.roll(s, 1, 1))
        s = s + jnp.where((lane & 2) == 0, pltpu.roll(s, L - 2, 1), pltpu.roll(s, 2, 1))
        scale = (0.5 + g_v[k, rows, :]) / (s + 1e-6)
        return jnp.concatenate([pq[:, j * L:(j + 1) * L] * scale for j in range(4)], axis=1)

    def ffn(t, carry):
        r0 = pl.multiple_of(t * HM, HM)
        rows = pl.ds(r0, HM)
        rp = pl.multiple_of(t * (HM // 2), HM // 2)
        HF = FC // 2
        nch = F // FC
        ha = jnp.concatenate([0.25 - 0.5 * g_v[0, rows, :]] * (HF // L), axis=1)
        hb = jnp.concatenate([0.25 - 0.5 * g_v[1, rows, :]] * (HF // L), axis=1)

        def act(gu, hs):
            g = gu[:, :HF]
            return (g * hs) * (1.0 + jnp.tanh(0.5 * g)) * gu[:, HF:]

        QM = HM // 2

        h_v[5, t, 0:8, 0:L] = jnp.zeros((8, L), F32)
        acc_v[49 + t, 0:8, :] = jnp.zeros((8, L), F32)
        mo_v[7 + t, 0:8, 0:L] = jnp.zeros((8, L), F32)
        seen = set()
        gv = []
        last = {}
        pending = []

        def leaf_terms(tab, i, j):
            return [(s1 * s2, (q1, q2)) for s1, q1 in tab[i] for s2, q2 in tab[j]]

        def queue(getl, getr, final=False, outers=ORD1):
            for i in outers:
                for j in ORD1:
                    pending.append((i, j, getl, getr, final))

        def issue(n):
            for _ in range(min(n, len(pending))):
                i, j, getl, getr, final = pending.pop(0)
                p = _dot(_term(leaf_terms(_LT, i, j), getl).astype(BF), _term(leaf_terms(_RT, i, j), getr).astype(BF))
                k = 7 * i + j
                if k in seen:
                    p = p + acc_v[k]
                seen.add(k)
                if final:
                    last[k] = p
                else:
                    acc_v[k] = p

        def geth(g):
            def get(q):
                q1, q2 = q
                return h_v[g, q1, (q2 // 2) * QM:(q2 // 2 + 1) * QM, (q2 % 2) * L:(q2 % 2 + 1) * L]
            return get

        def getm(q):
            q1, q2 = q
            r_ = (q1 // 2) * HD + (q2 // 2) * L
            c_ = (q1 % 2) * HD + (q2 % 2) * L
            return m_v[r_:r_ + L, c_:c_ + L]

        def getwd(g):
            def get(q):
                q1, q2 = q
                r_ = (2 * g + q2 // 2) * FC + (q1 // 2) * HF
                c_ = (q1 % 2) * HD + (q2 % 2) * L
                return wd_v[r_:r_ + HF, c_:c_ + L].astype(F32)
            return get

        for k in range(2):
            qk = qnorm(k, rows, HM)
            h_v[4, 2 * k] = qk[:, :HD]
            h_v[4, 2 * k + 1] = qk[:, HD:]
        queue(geth(4), getm)

        for c in range(nch):
            k1 = slice(c * FC, c * FC + HF)
            k2 = slice(c * FC + HF, (c + 1) * FC)
            rg = _rhs7(wg_v[:HD, k1], wg_v[:HD, k2], wg_v[HD:, k1], wg_v[HD:, k2])
            ru = _rhs7(wu_v[:HD, k1], wu_v[:HD, k2], wu_v[HD:, k1], wu_v[HD:, k2])
            rw = [jnp.concatenate([p, q], axis=1) for p, q in zip(rg, ru)]
            m = [None] * 7
            for n_, i in enumerate(ORD1):
                m[i] = _dot(_upk(lx_v[i, pl.ds(rp, HM // 2), :]), rw[i])
                issue(SCHED[c][n_])
            cqs = _comb(m)
            if GUARD:
                gv.append(_col_growth(m[0], _sub(cqs[0]), _sub(cqs[3]), DBG))
            for q, (cq, hs) in enumerate(zip(cqs, (ha, ha, hb, hb))):
                h_v[c // 2, q, :, (c % 2) * HF:(c % 2 + 1) * HF] = act(cq, hs)
            if c % 2 == 1:
                queue(geth(c // 2), getwd(c // 2), outers=ORD1 if c < nch - 2 else L2SET)
        assert not pending

        def l1(i, chunks, ks=slice(None)):
            ls, rs = [], []
            for c in chunks:
                ls.append(_term(_LT[i], lambda q: h_v[c // 2, q, ks, (c % 2) * HF:(c % 2 + 1) * HF]).astype(BF))
                rs.append(_term(_RT[i], lambda q: wd_v[c * FC + (q // 2) * HF:c * FC + (q // 2 + 1) * HF,
                                                       (q % 2) * HD:(q % 2 + 1) * HD].astype(F32)).astype(BF))
            return _dot(jnp.concatenate(ls, axis=1), jnp.concatenate(rs, axis=0))

        def leaves(i):
            c11, c12, c21, c22 = _comb([acc_v[7 * i + j] for j in range(7)])
            return jnp.concatenate([jnp.concatenate([c11, c12], axis=1), jnp.concatenate([c21, c22], axis=1)], axis=0)

        def chunks_of(i):
            return [nch - 1] if i in L2SET or i == FIRST else [nch - 3, nch - 2, nch - 1]

        def outer(i):
            base = mo_v[i] if i == FIRST else leaves(i)
            return base + l1(i, chunks_of(i))

        def emit(k, rk, c0, val):
            nr, nc = val.shape
            o_buf[k, pl.ds(rk, nr), c0:c0 + nc] = val.astype(BF)
            o_start(k, rk, nr, c0, nc)

        mo_v[FIRST] = leaves(FIRST) + l1(FIRST, [nch - 3, nch - 2])
        mo_v[2] = outer(2)
        m5 = outer(4)
        mo_v[4] = m5
        emit(0, r0, HD, mo_v[2] + m5)
        mo_v[1] = outer(1)
        m4 = outer(3)
        mo_v[3] = m4
        emit(1, r0, 0, mo_v[1] + m4)
        m1 = outer(0)
        mo_v[0] = m1
        o11 = (mo_v[0] + mo_v[3] - mo_v[4]) + outer(6)
        emit(0, r0, 0, o11)
        if GUARD:
            gl = functools.reduce(jnp.maximum, [_colmax(acc_v[7 * i]) for i in range(7)])
            chk_v[4:5, :] = jnp.maximum(chk_v[4:5, :], functools.reduce(jnp.maximum, gv))
            chk_v[5:6, :] = jnp.maximum(chk_v[5:6, :], jnp.maximum(_colmax(m1), jnp.concatenate([gl, gl], axis=1)))
            chk_v[6:7, :] = jnp.maximum(chk_v[6:7, :], _colmax(o11))
        mo_v[5] = mo_v[0] - mo_v[1] + mo_v[2] + leaves(5)
        k0 = 0
        for k, nr in enumerate(OC):
            ks = slice(k0, k0 + nr)
            res = mo_v[5, ks, :] + l1(5, chunks_of(5), ks)
            rk = pl.multiple_of(r0 + k0, L)
            if k < len(OC) - 1:
                emit(1, rk, HD, res)
            else:
                emit(1, rk, HD, res[:, :L])
                emit(1, rk, HD + L, res[:, L:])
            k0 += nr
        return carry

    with _scope("ffn", SC):
        lax.fori_loop(0, HS // HM, ffn, 0)
    if GUARD:
        ok = jnp.logical_and(jnp.max(chk_v[0:5, :]) <= 0.0,
                             jnp.max(chk_v[5:6, :]) <= KAPPA_OUT * jnp.max(chk_v[6:7, :]))
    with _scope("waito", SC):
        cp(o_buf, out_hbm, 0).wait()
    if DBG:
        o_buf[0, 0:16, 0:HD] = jnp.concatenate([chk_v[...], chk_v[...]], axis=0).astype(BF)
        cp(o_buf, out_hbm, 0).start()
        cp(o_buf, out_hbm, 0).wait()
        return
    if not GUARD:
        return

    @pl.when(jnp.logical_not(ok))
    def _classical():
        TR = 128
        nt = HS // TR

        def tile(i):
            return i // nt, pl.ds(pl.multiple_of((i % nt) * TR, TR), TR)

        def blk(b, base=0):
            return pl.ds(pl.multiple_of(base + b * L, L), L)

        def head_block(b, carry):
            fa_v[blk(b), :] = wqkv_v[:, blk(b, D)].astype(F32).T.astype(BF)
            m_v[0:L, :] = jnp.zeros((L, D), F32)

            def kbody(i, z):
                k, rows = tile(i)
                xt = x_v[k, rows, :]
                pkT = _phi(_dot_nt(fa_v[blk(b), :], xt))
                m_v[0:L, :] += _dot(pkT.astype(BF), xt)
                return z + pkT

            z = lax.fori_loop(0, 2 * nt, kbody, jnp.zeros((L, TR), F32))
            kv = jnp.where(same, _dot(m_v[0:L, :].astype(BF), wqkv_v[:, blk(b, 2 * D)]), 0.0).astype(BF)
            fa_v[blk(b), :] = _dot(kv, wo_v[blk(b), :]).astype(BF)
            z = jnp.broadcast_to(jnp.sum(z, axis=1, keepdims=True), (L, L))
            fz_v[b] = jnp.where(same, z, 0.0).astype(BF)
            return carry

        lax.fori_loop(0, D // L, head_block, 0)

        def obody(i, carry):
            k, rows = tile(i)
            m_v[0:TR, :] = jnp.zeros((TR, D), F32)

            def abody(b, c_):
                pq = _phi(_dot(x_v[k, rows, :], wqkv_v[:, blk(b)]))
                den = _dot(pq.astype(BF), fz_v[b]) + 1e-6
                m_v[0:TR, :] += _dot((pq * ((0.5 + g_v[k, rows, :]) / den)).astype(BF), fa_v[blk(b), :])
                return c_

            def fbody(c, c_):
                xt = x_v[k, rows, :]
                g = _dot(xt, wg_v[:, blk(c)])
                h = (g * (0.25 - 0.5 * g_v[k, rows, :])) * (1.0 + jnp.tanh(0.5 * g)) * _dot(xt, wu_v[:, blk(c)])
                m_v[0:TR, :] += _dot(h.astype(BF), wd_v[blk(c), :])
                return c_

            lax.fori_loop(0, D // L, abody, 0)
            lax.fori_loop(0, F // L, fbody, 0)
            o_buf[k, rows, :] = m_v[0:TR, :].astype(BF)
            return carry

        lax.fori_loop(0, 2 * nt, obody, 0)
        cp(o_buf, out_hbm, 0).start()
        cp(o_buf, out_hbm, 0).wait()


def impl(A_x, A_wqkv, A_wo, B_x, B_w_gate, B_w_up, B_w_down, gate_w,
         XS=(128, 640), KT=256, QT=256, HM=512, FC=256, OC=(256, 128, 128), ORD1=(2, 4, 1, 3, 0, 6, 5), L2SET=(2, 4, 1), FIRST=3,
         SCHED=((0, 0, 4, 4, 4, 4, 4), (4, 4, 4, 4, 4, 4, 5)) * 3 + ((0, 0, 4, 4, 4, 4, 5),),
         SC=False, GUARD=True, DBG=False):
    x = A_x.reshape(2, HS, D)
    any_spec = pl.BlockSpec(memory_space=pl.ANY)
    out = pl.pallas_call(
        functools.partial(_kernel, XS=XS, KT=KT, QT=QT, HM=HM, FC=FC, OC=OC, ORD1=ORD1, L2SET=L2SET, FIRST=FIRST, SCHED=SCHED, SC=SC, GUARD=GUARD, DBG=DBG),
        out_shape=jax.ShapeDtypeStruct((2, HS, D), BF),
        in_specs=[any_spec] * 7,
        out_specs=any_spec,
        scratch_shapes=[
            pltpu.VMEM((2, HS, D), BF),
            pltpu.VMEM((D, 3 * D), BF),
            pltpu.VMEM((D, D), BF),
            pltpu.VMEM((D, F), BF),
            pltpu.VMEM((D, F), BF),
            pltpu.VMEM((F, D), BF),
            pltpu.VMEM((D,), BF),
            pltpu.VMEM((7, HD // 2, HD), jnp.uint32),
            pltpu.VMEM((7, HD // 2, HD), jnp.uint32),
            pltpu.VMEM((7, HS // 2, HD), jnp.uint32),
            pltpu.VMEM((7, HD, HD), F32),
            pltpu.VMEM((D, L), F32),
            pltpu.VMEM((D, D), F32),
            pltpu.VMEM((6, 4, HM, HD), F32),
            pltpu.VMEM((51, HM // 2, L), F32),
            pltpu.VMEM((9, HM, HD), F32),
            pltpu.VMEM((8, D), F32),
            pltpu.VMEM((2, HS, D), F32),
            pltpu.VMEM((2, HS, L), F32),
            pltpu.VMEM((3, HD, L), F32),
            pltpu.VMEM((8, HD), F32),
            pltpu.VMEM((D, D), BF),
            pltpu.VMEM((D // L, L, L), BF),
            pltpu.VMEM((2, HS, D), BF),
            pltpu.SemaphoreType.DMA((3,)),
        ],
        compiler_params=pltpu.CompilerParams(vmem_limit_bytes=100 * 1024 * 1024, disable_bounds_checks=True,
                                             disable_semaphore_checks=True),
    )(x, A_wqkv, A_wo, B_w_gate, B_w_up, B_w_down, gate_w)
    return out.reshape(1, S, D)


@jax.jit
def pallas_gated_mix__linear_attn_block__swiglu_ffn__prompt_kernel(A_x, A_wqkv, A_wo, B_x, B_w_gate, B_w_up, B_w_down, gate_w):
    return impl(A_x, A_wqkv, A_wo, B_x, B_w_gate, B_w_up, B_w_down, gate_w)
```

```python
import functools

import jax
import jax.numpy as jnp
from jax import lax
import jax.experimental.pallas as pl
import jax.experimental.pallas.tpu as pltpu

S, D, F = 2048, 512, 1792
DH = 16
L = 128
HD, HS = D // 2, S // 2
HM = 512
QM = HM // 2
FC = 2 * L
NCH = F // FC
BF, F32 = jnp.bfloat16, jnp.float32

_LT = (((1, 0), (1, 3)), ((1, 2), (1, 3)), ((1, 0),), ((1, 3),), ((1, 0), (1, 1)), ((1, 2), (-1, 0)), ((1, 1), (-1, 3)))
_RT = (((1, 0), (1, 3)), ((1, 0),), ((1, 1), (-1, 3)), ((1, 2), (-1, 0)), ((1, 3),), ((1, 0), (1, 1)), ((1, 2), (1, 3)))
_CT = (((1, 0), (1, 3), (-1, 4), (1, 6)), ((1, 2), (1, 4)), ((1, 1), (1, 3)), ((1, 0), (-1, 1), (1, 2), (1, 5)))
_R_AS_L = (0, 2, 6, 5, 3, 4, 1)
_SET_A, _SET_B = (2, 4, 1, 3), (0, 6, 5)
_ORD = _SET_A + _SET_B

KAPPA = 16.0
KAPPA2 = 24.0
KAPPA_OUT = 4.0

_TILES = (0, 128, 256, 512, 768, 1024)
_P_ORD = (2, 4, 5, 3, 0, 1, 6)
_P_IN_K, _P_IN_Q = (2, 4, 1, 3, 0, 6), (3, 6, 5)
_Q_TILES = (2, 3, 4, 0, 1)
_GATE_AT = (1, 0)
_DOWN = (((4, 0, 6, 1, 5, 3, 2), (5, 6), _ORD),
         ((5, 1, 4, 0, 3, 2, 6), (5, 0, 6, 4), (4, 5, 0, 2, 3, 1, 6)),
         ((5, 1, 4, 0, 3, 2, 6), (5, 0, 6, 4), (4, 5, 0, 2, 3, 1, 6)),
         ((0, 4, 1, 2), (0, 4), _ORD))
_EXTRA = ((8, 8, 0, 4, 4, 4, 4), (8, 8, 8, 4, 4, 4, 0), (8, 8, 8, 4, 4, 4, 0), (8, 4, 0, 4, 4, 0, 2))


def _phi(t):
    return jnp.where(t > 0, t + 1.0, jnp.exp(t)) + 1e-6


def _dot(a, b):
    return jnp.dot(a, b, preferred_element_type=F32)


def _dot_nt(a, b):
    return lax.dot_general(a, b, (((1,), (1,)), ((), ())), preferred_element_type=F32)


def _swap_lane_bit(a, b, k):
    lane = lax.broadcasted_iota(jnp.int32, a.shape, 1)
    lo = (lane & k) == 0
    return jnp.where(lo, a, pltpu.roll(b, k, 1)), jnp.where(lo, pltpu.roll(a, L - k, 1), b)


def _perm_lanes(blocks):
    b0, b1, b2, b3 = blocks
    b0, b2 = _swap_lane_bit(b0, b2, 8)
    b1, b3 = _swap_lane_bit(b1, b3, 8)
    b0, b1 = _swap_lane_bit(b0, b1, 4)
    b2, b3 = _swap_lane_bit(b2, b3, 4)
    return [b0, b1, b2, b3]


def _term(terms, get):
    v = get(terms[0][1])
    for sg, q in terms[1:]:
        v = v + get(q) if sg > 0 else v - get(q)
    return v


def _operand(terms, get):
    return get(terms[0][1]) if len(terms) == 1 else _term(terms, lambda q: get(q).astype(F32)).astype(BF)


def _leaf_terms(tab, i, j):
    return [(s1 * s2, (q1, q2)) for s1, q1 in tab[i] for s2, q2 in tab[j]]


def _strassen_step(i, v, get, put, fin):
    if i == 2:
        put(0, v)
    elif i == 4:
        put(1, v)
        fin(1, v + get(0))
    elif i == 1:
        put(2, v)
    elif i == 3:
        fin(2, v + get(2))
        put(1, v - get(1))
    elif i == 0:
        put(3, v)
    elif i == 6:
        fin(0, (v + get(1)) + get(3))
    else:
        fin(3, ((v + get(0)) - get(2)) + get(3))


def _colmax(v):
    return jnp.max(jnp.abs(v), axis=0, keepdims=True)


def _colsum(v):
    return jnp.sum(jnp.abs(v), axis=0, keepdims=True)


def _lanefold(v, op):
    r = v[:, 0:L]
    for j in range(1, v.shape[1] // L):
        r = op(r, v[:, j * L:(j + 1) * L])
    return r


def _body(x_hbm, wqkv_hbm, wo_hbm, wg_hbm, wu_hbm, wd_hbm, gw_hbm, out_hbm,
          x_v, wqkv_v, wo_v, wg_v, wu_v, wd_v, gw_v, gf_v, wq_v, go_v, rt_v, p_acc, z_acc, m_v, h_v, acc_v, mo_v,
          pq_v, g_v, ks_v, chk_v, fa_v, fz_v, o_buf, sem):
    def cp(src, dst, k):
        return pltpu.make_async_copy(src, dst, sem.at[k])

    def xcp(a, b, k):
        return cp(x_hbm.at[:, pl.ds(a, b - a), :], x_v.at[:, pl.ds(a, b - a), :], k)

    def wcp(r0, nr, c0, k):
        return cp(wqkv_hbm.at[pl.ds(r0, nr), pl.ds(c0, D)], wqkv_v.at[pl.ds(r0, nr), pl.ds(c0, D)], k)

    g1 = [wcp(0, HD, D, 0)]
    g2 = [wcp(HD, HD, D, 1)]
    g3 = [xcp(0, _TILES[1], 2)]
    g4 = [xcp(_TILES[1], _TILES[3], 0)]
    g5 = [xcp(_TILES[3], HS, 1), wcp(0, D, 0, 1), wcp(0, D, 2 * D, 1), cp(wo_hbm, wo_v, 1), cp(gw_hbm, gw_v, 1)]
    g6 = [cp(wg_hbm, wg_v, 2), cp(wu_hbm, wu_v, 2), cp(wd_hbm, wd_v, 2)]

    def start(g):
        for c in g:
            c.start()

    def wait(g):
        for c in g:
            c.wait()

    rk = [None] * 7
    lxs = {}

    def lx(t, i):
        if (t, i) not in lxs:
            lxs[t, i] = _operand(_LT[i], lambda q: x_v[q // 2, _TILES[t]:_TILES[t + 1], (q % 2) * HD:(q % 2 + 1) * HD])
        return lxs[t, i]

    def acc(ref, idx, v, op, first):
        ref[idx] = v if first else op(v, ref[idx])

    def kprod(t, i):
        n = _TILES[t + 1] - _TILES[t]
        v = _dot_nt(rk[i], lx(t, i))
        if i == 0:
            acc(ks_v, 0, _lanefold(jnp.abs(v), jnp.maximum), jnp.maximum, t == 0)

        def put(k, u):
            mo_v[k, 0:HD, 0:n] = u

        def fin(q, c):
            if q in (0, 3):
                acc(ks_v, 1 + q // 3, _lanefold(jnp.abs(c), jnp.add), jnp.add, t == 0)
            p = _phi(c)
            h_v[t % 4, (0, 2, 1, 3)[q], 0:HD, 0:n] = p
            acc(z_acc, (slice((q % 2) * HD, (q % 2 + 1) * HD),), _lanefold(p, jnp.add), jnp.add, t == 0 and q in (1, 2))

        _strassen_step(i, v, lambda k: mo_v[k, 0:HD, 0:n], put, fin)

    def pprod(t, i):
        n = _TILES[t + 1] - _TILES[t]
        l = _term(_LT[i], lambda q: h_v[t % 4, q, 0:HD, 0:n]).astype(BF)
        acc(p_acc, i, _dot(l, lx(t, _R_AS_L[i])), jnp.add, t == 0)

    start(g1)
    start(g2)
    start(g3)
    wait(g1)
    start(g4)
    ta = wqkv_v[:HD, D:2 * D].astype(F32).T
    rk[1] = ta[:HD].astype(BF)
    rk[5] = (ta[:HD] + ta[HD:]).astype(BF)
    wait(g2)
    start(g5)
    tb = wqkv_v[HD:, D:2 * D].astype(F32).T
    rk[0] = (ta[:HD] + tb[HD:]).astype(BF)
    rk[2] = (ta[HD:] - tb[HD:]).astype(BF)
    rk[3] = (tb[:HD] - ta[:HD]).astype(BF)
    rk[4] = tb[HD:].astype(BF)
    rk[6] = (tb[:HD] + tb[HD:]).astype(BF)
    wait(g3)
    start(g6)
    for i in _ORD:
        kprod(0, i)
    for i in _P_ORD:
        pprod(0, i)
    wait(g4)
    for i in _ORD:
        kprod(1, i)
    for i, j in zip(_ORD, _P_ORD):
        kprod(2, i)
        pprod(1, j)
    for i in _P_ORD:
        pprod(2, i)
    wait(g5)
    gf_v[...] = jnp.broadcast_to(gw_v[...].astype(F32).reshape(1, D), (8, D))
    blocks = _perm_lanes([pltpu.bitcast(wqkv_v[:, j * L:(j + 1) * L], jnp.uint32) for j in range(4)])
    for j in range(4):
        wq_v[0:HD, j * L:(j + 1) * L] = blocks[j]
    for i in _ORD:
        kprod(3, i)
    p_jobs = [(t, i) for t in (3, 4) for i in _P_ORD]
    for i in _ORD:
        kprod(4, i)
        if i in _P_IN_K:
            pprod(*p_jobs.pop(0))

    zrow = jnp.sum(z_acc[...].T, axis=0, keepdims=True)
    zb = _perm_lanes([jnp.broadcast_to(zrow[:, j * L:(j + 1) * L], (8, L)) for j in range(4)])
    zr = jnp.concatenate(zb, axis=1)[0:1, :]
    rqs = {}
    qs = {}
    q_growth = []

    def rq(i):
        if i not in rqs:
            rqs[i] = _operand(_RT[i], lambda q: pltpu.bitcast(
                wq_v[(q // 2) * L:(q // 2 + 1) * L, (q % 2) * HD:(q % 2 + 1) * HD], BF))
        return rqs[i]

    def gate(k, rows):
        gl = jnp.sum(x_v[k, rows, :].astype(F32) * gf_v[...][0:1, :], axis=1, keepdims=True)
        th = jnp.broadcast_to(jnp.tanh(0.5 * gl), (rows.stop - rows.start, L))
        hs = 0.25 - 0.25 * th
        g_v[k, rows, :] = hs
        if rows.start < HM:
            h_v[4, k, rows, 0:L] = hs
        return 0.5 + 0.5 * th

    def qprod(t, i):
        rows = slice(_TILES[t], _TILES[t + 1])
        n = _TILES[t + 1] - _TILES[t]
        v = _dot(lx(t, i), rq(i))
        if i == 0:
            qs["g"] = _colmax(v)
        if i in _GATE_AT:
            gf_v[1:2, :] = jnp.concatenate([v[0:1, :], v[0:1, :]], axis=1)
            qs["gate", _GATE_AT.index(i)] = gate(_GATE_AT.index(i), rows)

        def put(k, u):
            mo_v[k, HD:HD + n, :] = u

        def fin(q, c):
            k, cols = q // 2, slice((q % 2) * HD, (q % 2 + 1) * HD)
            if q in (0, 3):
                qs[q] = _colsum(c[:L])
                if q == 3:
                    q_growth.append(qs["g"] - (KAPPA / L) * jnp.minimum(qs[0], qs[3]))
            pq = _phi(c)
            s = _lanefold(pq * zr[:, cols], jnp.add)
            if q in (1, 2):
                pq_v[k, rows, cols] = pq
                mo_v[4 + k, 0:n, 0:L] = s
                return
            s = s + mo_v[4 + k, 0:n, 0:L]
            lane = lax.broadcasted_iota(jnp.int32, (n, L), 1)
            s = s + jnp.where((lane & 1) == 0, pltpu.roll(s, L - 1, 1), pltpu.roll(s, 1, 1))
            s = s + jnp.where((lane & 2) == 0, pltpu.roll(s, L - 2, 1), pltpu.roll(s, 2, 1))
            den = s + 1e-6
            inv = pl.reciprocal(den, approx=True)
            inv = inv * (2.0 - den * inv)
            scale = qs["gate", k] * inv
            scale = jnp.concatenate([scale, scale], axis=1)
            other = slice(HD - cols.start, 2 * HD - cols.start)
            pq_v[k, rows, cols] = pq * scale
            pq_v[k, rows, other] = pq_v[k, rows, other] * scale

        _strassen_step(i, v, lambda k: mo_v[k, HD:HD + n, :], put, fin)

    pprod(*p_jobs.pop(0))
    for t in _Q_TILES:
        for i in _ORD:
            qprod(t, i)
            if i in _P_IN_Q and p_jobs:
                pprod(*p_jobs.pop(0))
    assert not p_jobs

    same = (lax.broadcasted_iota(jnp.int32, (L, L), 0) // DH) == (lax.broadcasted_iota(jnp.int32, (L, L), 1) // DH)
    kvs = []
    pdiag = []
    for b in range(D // L):
        rs = slice((b % 2) * L, (b % 2 + 1) * L)
        pb = [_term(_CT[2 * (b // 2) + c], lambda j: p_acc[j, rs, :]) for c in range(2)]
        pdiag.append(pb[b // 2])
        kv = _dot(jnp.concatenate(pb, axis=1).astype(BF), wqkv_v[:, 2 * D + b * L: 2 * D + (b + 1) * L])
        kvs.append(jnp.where(same, kv, 0.0).astype(BF))
    p11, p22 = jnp.concatenate(pdiag[:2], axis=0), jnp.concatenate(pdiag[2:], axis=0)
    sub_lo = lax.broadcasted_iota(jnp.int32, (16, 8, HD), 1) < 4
    for b1 in range(2):
        for c in range(2):
            cols = slice(c * HD, (c + 1) * HD)
            u, v = [_dot(kvs[b], wo_v[b * L:(b + 1) * L, cols]).reshape(16, 8, HD) for b in (2 * b1, 2 * b1 + 1)]
            for d2, w in enumerate((jnp.where(sub_lo, u, pltpu.roll(v, 4, 1)), jnp.where(sub_lo, pltpu.roll(u, 4, 1), v))):
                for e in range(16):
                    r = (2 * (e % 2) + d2) * L + (e // 2) * 16 + b1 * 8
                    m_v[r:r + 8, cols] = w[e]

    pm = p_acc[0]
    chk_v[0:1, :] = functools.reduce(jnp.maximum, q_growth)
    chk_v[1:2, :] = _colmax(pm) - (KAPPA / HD) * jnp.minimum(_colsum(p11), _colsum(p22))
    stats = ((_lanefold(jnp.abs(pm), jnp.maximum), _lanefold(jnp.abs(p11), jnp.add), _lanefold(jnp.abs(p22), jnp.add), HD),
             (ks_v[0], ks_v[1], ks_v[2], HS))
    for r, (kg, k1, k2, n) in enumerate(stats):
        kt = jnp.minimum(jnp.sum(k1, axis=1, keepdims=True), jnp.sum(k2, axis=1, keepdims=True))
        km = jnp.max(kg - (KAPPA / n) * kt, axis=0, keepdims=True)
        chk_v[2 + r:3 + r, :] = jnp.concatenate([km, km], axis=1)
    chk_v[4:8, :] = jnp.zeros((4, HD), F32)

    wait(g6)

    def ffn(t, carry):
        r0 = pl.multiple_of(t * HM, HM)

        h_v[5, t, 0:8, 0:L] = jnp.zeros((8, L), F32)
        acc_v[49 + t, 0:8, :] = jnp.zeros((8, L), F32)
        mo_v[7 + t, 0:8, 0:L] = jnp.zeros((8, L), F32)
        p_acc[7 + t, 0:8, 0:L] = jnp.zeros((8, L), F32)
        gf_v[pl.ds(2 + t, 1), :] = jnp.zeros((1, D), F32)
        wq_v[pl.ds(pl.multiple_of(HD + 8 * t, 8), 8), 0:L] = jnp.zeros((8, L), jnp.uint32)
        go_v[7 + t, 0, 0, 0:8, :] = jnp.zeros((8, L), F32)
        rt_v[2 + t, 0, 0, 0:8, :] = jnp.zeros((8, L), F32)

        seen = set()
        singles = []
        sets = []

        def queue(getl, getr, outers, whole, order):
            for i in outers:
                if i in whole:
                    sets.append((i, _SET_A, getl, getr))
                    sets.append((i, _SET_B, getl, getr))
                else:
                    for j in order:
                        singles.append((i, j, getl, getr))

        def put_leaf(i, j, p):
            k = 7 * i + j
            acc_v[k] = p + acc_v[k] if k in seen else p
            seen.add(k)

        def single(n):
            for _ in range(min(n, len(singles))):
                i, j, getl, getr = singles.pop(0)
                put_leaf(i, j, _dot(_term(_leaf_terms(_LT, i, j), getl).astype(BF),
                                    _term(_leaf_terms(_RT, i, j), getr).astype(BF)))

        def issue(n):
            if n % 4:
                single(n)
                return
            for _ in range(n // 4):
                if not sets:
                    single(4)
                    continue
                i, js, getl, getr = sets.pop(0)
                lo = [_term(_LT[i], lambda q1: getl((q1, q2))) for q2 in range(4)]
                ro = [_term(_RT[i], lambda q1: getr((q1, q2))) for q2 in range(4)]
                for j in js:
                    put_leaf(i, j, _dot(_term(_LT[j], lambda q: lo[q]).astype(BF), _term(_RT[j], lambda q: ro[q]).astype(BF)))
                single(4 - len(js))

        def geth(g, q):
            q1, q2 = q
            return h_v[g, q1, (q2 // 2) * QM:(q2 // 2 + 1) * QM, (q2 % 2) * L:(q2 % 2 + 1) * L]

        def getwd(g, q):
            q1, q2 = q
            r = (2 * g + q2 // 2) * FC + (q1 // 2) * L
            c = (q1 % 2) * HD + (q2 % 2) * L
            return wd_v[r:r + L, c:c + L].astype(F32)

        def getq(q):
            q1, q2 = q
            c = (q1 % 2) * HD + (q2 % 2) * L
            return pq_v[q1 // 2, (q2 // 2) * QM:(q2 // 2 + 1) * QM, c:c + L]

        def getm(q):
            q1, q2 = q
            r = (q1 // 2) * HD + (q2 // 2) * L
            c = (q1 % 2) * HD + (q2 % 2) * L
            return m_v[r:r + L, c:c + L]

        queue(getq, getm, *_DOWN[0])

        l2 = {}
        growth = []

        def xblk(q1, q2):
            c = (q1 % 2) * HD + (q2 % 2) * L
            return x_v[q1 // 2, pl.ds(pl.multiple_of(r0 + (q2 // 2) * QM, QM), QM), c:c + L]

        def gate_up(g):
            half = g == NCH // 2
            mats = (0,) if half else (1, 0)
            gmax = {}
            tmin = {}

            def wblk(w, q1, q2):
                r = (q1 // 2) * HD + (q2 // 2) * L
                c = (2 * g + (0 if half else q2 % 2)) * FC + (q1 % 2) * L
                return (wg_v, wu_v)[q2 % 2 if half else w][r:r + L, c:c + L]

            def fin(w, q2, q1, c):
                if q1 in (0, 3) and q2 in (0, 3):
                    v = _colsum(c.reshape(QM // 16, 2, 8, L)[:, 0].reshape(QM // 2, L))
                    tmin[w] = jnp.minimum(tmin[w], v) if w in tmin else v
                c2 = 0 if half else q2 % 2
                dst = (g, q1, slice((q2 // 2) * QM, (q2 // 2 + 1) * QM), slice(c2 * L, (c2 + 1) * L))
                first = q2 in (1, 2) if half else w == 1
                is_gate = q2 % 2 == 0 if half else w == 0
                o = h_v[4, q1 // 2, (q2 // 2) * QM:(q2 // 2 + 1) * QM, 0:L] if first else h_v[dst]
                h_v[dst] = (c * o) * (1.0 + jnp.tanh(0.5 * c)) if is_gate else c * o

            for n, i in enumerate(_ORD):
                shared = len(_RT[i]) > 1
                if shared:
                    for w in mats:
                        for q2 in range(4):
                            rt_v[n % 2, w, q2] = _term(_RT[i], lambda q1: wblk(w, q1, q2).astype(F32))

                def leaves(w, js):
                    if (i, js[0]) not in l2:
                        xq = [_term(_LT[i], lambda q1: xblk(q1, q2).astype(F32)) for q2 in range(4)]
                        for j in js:
                            terms = _leaf_terms(_LT, i, j)
                            l2[i, j] = xblk(*terms[0][1]) if len(terms) == 1 else _term(_LT[j], lambda q2: xq[q2]).astype(BF)
                    out = []
                    for j in js:
                        if shared:
                            r = _term(_RT[j], lambda q2: rt_v[n % 2, w, q2]).astype(BF)
                        else:
                            r = _operand(_RT[j], lambda q2: wblk(w, _RT[i][0][1], q2))
                        out.append(_dot(l2[i, j], r))
                    return out

                def done(w, q2, v):
                    def put(k, u):
                        go_v[k, w, q2] = u

                    _strassen_step(i, v, lambda k: go_v[k, w, q2], put, functools.partial(fin, w, q2))

                for w in mats:
                    m3, m5, m2, m4 = leaves(w, _SET_A)
                    go_v[4, w, 0] = m4 - m5
                    go_v[4, w, 3] = m3 - m2
                    done(w, 1, m3 + m5)
                    done(w, 2, m2 + m4)
                    m1, m7, m6 = leaves(w, _SET_B)
                    issue(1)
                    for v in {0: (m1, m7, m6), 5: (m1,), 6: (m1,)}.get(i, ()):
                        v = _colmax(v)
                        gmax[w] = jnp.maximum(gmax[w], v) if w in gmax else v
                    done(w, 0, (m1 + m7) + go_v[4, w, 0])
                    done(w, 3, (m1 + m6) + go_v[4, w, 3])
                issue(_EXTRA[g][n])
            gm = jnp.concatenate([gmax[0], gmax[mats[0]]], axis=1)
            tm = jnp.concatenate([tmin[0], tmin[mats[0]]], axis=1)
            growth.append(gm - (KAPPA2 / (QM // 2)) * tm)

        for g in range(NCH // 2 + 1):
            gate_up(g)
            if g < NCH // 2:
                queue(functools.partial(geth, g), functools.partial(getwd, g), *_DOWN[g + 1])
        assert not singles and not sets
        pq_v[:, 0:HM, :] = pq_v[:, HM:2 * HM, :]
        for k in range(2):
            h_v[4, k, :, 0:L] = g_v[k, HM:2 * HM, :]

        def rest(i, chunks, ks=slice(None)):
            ls = [_term(_LT[i], lambda q: h_v[c // 2, q, ks, (c % 2) * L:(c % 2 + 1) * L]) for c in chunks]
            rs = [_term(_RT[i], lambda q: wd_v[c * FC + (q // 2) * L:c * FC + (q // 2 + 1) * L,
                                               (q % 2) * HD:(q % 2 + 1) * HD].astype(F32)) for c in chunks]
            return _dot(jnp.concatenate(ls, axis=1).astype(BF), jnp.concatenate(rs, axis=0).astype(BF))

        def outer(i, chunks=None, k0=0, nr=HM):
            if chunks is None:
                chunks = [NCH - 1] if i in _DOWN[3][0] else [NCH - 3, NCH - 2, NCH - 1]
            v = rest(i, chunks, slice(k0, k0 + nr))
            n = min(nr, QM)
            out = []
            for a in range(k0, k0 + nr, n):
                cols = []
                for c2 in range(2):
                    u = v[a - k0:a - k0 + n, c2 * L:(c2 + 1) * L]
                    for sg, j in _CT[2 * (a // QM) + c2]:
                        p = acc_v[7 * i + j, a % QM:a % QM + n, :]
                        u = u + p if sg > 0 else u - p
                    cols.append(u)
                out.append(jnp.concatenate(cols, axis=1))
            return jnp.concatenate(out, axis=0)

        def emit(k, k0, c0, val):
            nr, nc = val.shape
            rows = pl.ds(pl.multiple_of(r0 + k0, nr), nr)
            o_buf[k, rows, c0:c0 + nc] = val.astype(BF)
            cp(o_buf.at[k, rows, pl.ds(c0, nc)], out_hbm.at[k, rows, pl.ds(c0, nc)], 0).start()

        mo_v[3] = outer(3, [NCH - 3, NCH - 2])
        mo_v[2] = outer(2)
        m5 = outer(4)
        mo_v[4] = m5
        emit(0, 0, HD, m5 + mo_v[2])
        mo_v[1] = outer(1)
        m4 = rest(3, [NCH - 1]) + mo_v[3]
        mo_v[3] = m4 - mo_v[4]
        emit(1, 0, 0, m4 + mo_v[1])
        m1 = outer(0)
        mo_v[3] = m1 + mo_v[3]
        mo_v[5] = (m1 - mo_v[1]) + mo_v[2]
        for k0 in range(0, HM, QM):
            o11 = outer(6, None, k0, QM) + mo_v[3, k0:k0 + QM, :]
            emit(0, k0, 0, o11)
        gl = functools.reduce(jnp.maximum, [_colmax(acc_v[7 * i]) for i in (0, 5, 6)])
        chk_v[4:5, :] = jnp.maximum(chk_v[4:5, :], functools.reduce(jnp.maximum, growth))
        chk_v[5:6, :] = jnp.maximum(chk_v[5:6, :], jnp.maximum(_colmax(m1), jnp.concatenate([gl, gl], axis=1)))
        chk_v[6:7, :] = jnp.maximum(chk_v[6:7, :], _colmax(o11))
        for k0, nr, piece in ((0, QM, QM), (QM, L, L), (QM + L, L, L // 2)):
            res = outer(5, None, k0, nr) + mo_v[5, k0:k0 + nr, :]
            for e in range(0, nr, piece):
                emit(1, k0 + e, HD, res[e:e + piece])
        return carry

    lax.fori_loop(0, HS // HM, ffn, 0)
    omax = jnp.max(chk_v[6:7, :])
    ok = jnp.logical_and(jnp.max(chk_v[0:5, :]) <= 0.0, jnp.max(chk_v[5:6, :]) <= KAPPA_OUT * omax)
    cp(o_buf, out_hbm, 0).wait()

    @pl.when(jnp.logical_not(ok))
    def _classical():
        nt = HS // L

        def tile(i):
            return i // nt, pl.ds(pl.multiple_of((i % nt) * L, L), L)

        def blk(b, base=0):
            return pl.ds(pl.multiple_of(base + b * L, L), L)

        def head_block(b, carry):
            fa_v[blk(b), :] = wqkv_v[:, blk(b, D)].astype(F32).T.astype(BF)
            m_v[0:L, :] = jnp.zeros((L, D), F32)

            def kbody(i, z):
                k, rows = tile(i)
                xt = x_v[k, rows, :]
                pkt = _phi(_dot_nt(fa_v[blk(b), :], xt))
                m_v[0:L, :] += _dot(pkt.astype(BF), xt)
                return z + pkt

            z = lax.fori_loop(0, 2 * nt, kbody, jnp.zeros((L, L), F32))
            kv = jnp.where(same, _dot(m_v[0:L, :].astype(BF), wqkv_v[:, blk(b, 2 * D)]), 0.0).astype(BF)
            fa_v[blk(b), :] = _dot(kv, wo_v[blk(b), :]).astype(BF)
            z = jnp.broadcast_to(jnp.sum(z, axis=1, keepdims=True), (L, L))
            fz_v[b] = jnp.where(same, z, 0.0).astype(BF)
            return carry

        lax.fori_loop(0, D // L, head_block, 0)

        def obody(i, carry):
            k, rows = tile(i)
            m_v[0:L, :] = jnp.zeros((L, D), F32)

            def abody(b, c):
                pq = _phi(_dot(x_v[k, rows, :], wqkv_v[:, blk(b)]))
                den = _dot(pq.astype(BF), fz_v[b]) + 1e-6
                m_v[0:L, :] += _dot((pq * ((1.0 - 2.0 * g_v[k, rows, :]) / den)).astype(BF), fa_v[blk(b), :])
                return c

            def fbody(f, c):
                xt = x_v[k, rows, :]
                g = _dot(xt, wg_v[:, blk(f)])
                h = (g * g_v[k, rows, :]) * (1.0 + jnp.tanh(0.5 * g)) * _dot(xt, wu_v[:, blk(f)])
                m_v[0:L, :] += _dot(h.astype(BF), wd_v[blk(f), :])
                return c

            lax.fori_loop(0, D // L, abody, 0)
            lax.fori_loop(0, F // L, fbody, 0)
            o_buf[k, rows, :] = m_v[0:L, :].astype(BF)
            return carry

        lax.fori_loop(0, 2 * nt, obody, 0)
        cp(o_buf, out_hbm, 0).start()
        cp(o_buf, out_hbm, 0).wait()

    return omax < 0.0


def _kernel(*refs):
    lax.while_loop(lambda again: again, lambda _: _body(*refs), jnp.bool_(True))


@jax.jit
def pallas_gated_mix__linear_attn_block__swiglu_ffn__prompt_kernel(
    A_x: jax.Array,
    A_wqkv: jax.Array,
    A_wo: jax.Array,
    B_x: jax.Array,
    B_w_gate: jax.Array,
    B_w_up: jax.Array,
    B_w_down: jax.Array,
    gate_w: jax.Array,
):
    del B_x
    hbm = pl.BlockSpec(memory_space=pl.ANY)
    out = pl.pallas_call(
        _kernel,
        out_shape=jax.ShapeDtypeStruct((2, HS, D), BF),
        in_specs=[hbm] * 7,
        out_specs=hbm,
        scratch_shapes=[
            pltpu.VMEM((2, HS, D), BF),
            pltpu.VMEM((D, 3 * D), BF),
            pltpu.VMEM((D, D), BF),
            pltpu.VMEM((D, F), BF),
            pltpu.VMEM((D, F), BF),
            pltpu.VMEM((F, D), BF),
            pltpu.VMEM((D,), BF),
            pltpu.VMEM((8, D), F32),
            pltpu.VMEM((HD + 16, D), jnp.uint32),
            pltpu.VMEM((9, 2, 4, QM, L), F32),
            pltpu.VMEM((4, 2, 4, L, L), F32),
            pltpu.VMEM((9, HD, HD), F32),
            pltpu.VMEM((D, L), F32),
            pltpu.VMEM((D, D), F32),
            pltpu.VMEM((6, 4, HM, HD), F32),
            pltpu.VMEM((51, QM, L), F32),
            pltpu.VMEM((9, HM, HD), F32),
            pltpu.VMEM((2, HS, D), F32),
            pltpu.VMEM((2, HS, L), F32),
            pltpu.VMEM((3, HD, L), F32),
            pltpu.VMEM((8, HD), F32),
            pltpu.VMEM((D, D), BF),
            pltpu.VMEM((D // L, L, L), BF),
            pltpu.VMEM((2, HS, D), BF),
            pltpu.SemaphoreType.DMA((3,)),
        ],
        compiler_params=pltpu.CompilerParams(
            vmem_limit_bytes=100 * 1024 * 1024,
            disable_bounds_checks=True,
            disable_semaphore_checks=True,
        ),
    )(A_x.reshape(2, HS, D), A_wqkv, A_wo, B_w_gate, B_w_up, B_w_down, gate_w)
    return out.reshape(1, S, D)
```

```python
import functools

import jax
import jax.numpy as jnp
from jax import lax
import jax.experimental.pallas as pl
import jax.experimental.pallas.tpu as pltpu

S, D, F = 2048, 512, 1792
DH = 16
L = 128
HD, HS = D // 2, S // 2
HM = 512
QM = HM // 2
FC = 2 * L
NCH = F // FC
BF, F32 = jnp.bfloat16, jnp.float32

_LT = (((1, 0), (1, 3)), ((1, 2), (1, 3)), ((1, 0),), ((1, 3),), ((1, 0), (1, 1)), ((1, 2), (-1, 0)), ((1, 1), (-1, 3)))
_RT = (((1, 0), (1, 3)), ((1, 0),), ((1, 1), (-1, 3)), ((1, 2), (-1, 0)), ((1, 3),), ((1, 0), (1, 1)), ((1, 2), (1, 3)))
_CT = (((1, 0), (1, 3), (-1, 4), (1, 6)), ((1, 2), (1, 4)), ((1, 1), (1, 3)), ((1, 0), (-1, 1), (1, 2), (1, 5)))
_R_AS_L = (0, 2, 6, 5, 3, 4, 1)
_SET_A, _SET_B = (2, 4, 1, 3), (0, 6, 5)
_ORD = _SET_A + _SET_B

KAPPA = 16.0
KAPPA2 = 24.0
KAPPA_OUT = 4.0

_TILES = (0, 128, 256, 512, 768, 1024)
_P_ORD = (2, 4, 5, 3, 0, 1, 6)
_P_IN_K, _P_IN_Q = (2, 4, 1, 3, 0, 6), (3, 6, 5)
_Q_TILES = (2, 3, 4, 0, 1)
_GATE_AT = (1, 0)
_DOWN = (((1, 6, 0, 2, 3, 4, 5), (5,), _ORD),
         ((5, 1, 4, 0, 3, 2, 6), (5, 0, 6, 4), (4, 5, 0, 2, 3, 1, 6)),
         ((5, 1, 4, 0, 3, 2, 6), (5, 0, 6, 4), (4, 5, 0, 2, 3, 1, 6)),
         ((4, 1, 0, 2), (0, 1), _ORD))
_EXTRA = ((0, 8, 4, 4, 4, 4, 4), (8, 8, 8, 4, 4, 4, 0), (8, 8, 8, 4, 4, 4, 0), (8, 0, 4, 0, 4, 4, 2))


def _phi(t):
    return jnp.where(t > 0, t + 1.0, jnp.exp(t)) + 1e-6


def _dot(a, b):
    return jnp.dot(a, b, preferred_element_type=F32)


def _dot_nt(a, b):
    return lax.dot_general(a, b, (((1,), (1,)), ((), ())), preferred_element_type=F32)


def _swap_lane_bit(a, b, k):
    lane = lax.broadcasted_iota(jnp.int32, a.shape, 1)
    lo = (lane & k) == 0
    return jnp.where(lo, a, pltpu.roll(b, k, 1)), jnp.where(lo, pltpu.roll(a, L - k, 1), b)


def _perm_lanes(blocks):
    b0, b1, b2, b3 = blocks
    b0, b2 = _swap_lane_bit(b0, b2, 8)
    b1, b3 = _swap_lane_bit(b1, b3, 8)
    b0, b1 = _swap_lane_bit(b0, b1, 4)
    b2, b3 = _swap_lane_bit(b2, b3, 4)
    return [b0, b1, b2, b3]


def _term(terms, get):
    v = get(terms[0][1])
    for sg, q in terms[1:]:
        v = v + get(q) if sg > 0 else v - get(q)
    return v


def _operand(terms, get):
    return get(terms[0][1]) if len(terms) == 1 else _term(terms, lambda q: get(q).astype(F32)).astype(BF)


def _leaf_terms(tab, i, j):
    return [(s1 * s2, (q1, q2)) for s1, q1 in tab[i] for s2, q2 in tab[j]]


def _strassen_step(i, v, get, put, fin):
    if i == 2:
        put(0, v)
    elif i == 4:
        put(1, v)
        fin(1, v + get(0))
    elif i == 1:
        put(2, v)
    elif i == 3:
        fin(2, v + get(2))
        put(1, v - get(1))
    elif i == 0:
        put(3, v)
    elif i == 6:
        fin(0, (v + get(1)) + get(3))
    else:
        fin(3, ((v + get(0)) - get(2)) + get(3))


def _colmax(v):
    return jnp.max(jnp.abs(v), axis=0, keepdims=True)


def _colsum(v):
    return jnp.sum(jnp.abs(v), axis=0, keepdims=True)


def _lanefold(v, op):
    r = v[:, 0:L]
    for j in range(1, v.shape[1] // L):
        r = op(r, v[:, j * L:(j + 1) * L])
    return r


def _body(x_hbm, wqkv_hbm, wo_hbm, wg_hbm, wu_hbm, wd_hbm, gw_hbm, out_hbm,
          x_v, wqkv_v, wo_v, wg_v, wu_v, wd_v, gw_v, gf_v, wq_v, go_v, rt_v, p_acc, z_acc, m_v, h_v, acc_v, mo_v,
          pq_v, g_v, ks_v, chk_v, fa_v, fz_v, o_buf, sem):
    def cp(src, dst, k):
        return pltpu.make_async_copy(src, dst, sem.at[k])

    def xcp(a, b, k):
        return cp(x_hbm.at[:, pl.ds(a, b - a), :], x_v.at[:, pl.ds(a, b - a), :], k)

    def wcp(r0, nr, c0, k):
        return cp(wqkv_hbm.at[pl.ds(r0, nr), pl.ds(c0, D)], wqkv_v.at[pl.ds(r0, nr), pl.ds(c0, D)], k)

    g1 = [wcp(0, HD, D, 0)]
    g2 = [wcp(HD, HD, D, 1)]
    g3 = [xcp(0, _TILES[1], 2)]
    g4 = [xcp(_TILES[1], _TILES[3], 0)]
    g5 = [xcp(_TILES[3], HS, 1), wcp(0, D, 0, 1), wcp(0, D, 2 * D, 1), cp(wo_hbm, wo_v, 1), cp(gw_hbm, gw_v, 1)]
    g6 = [cp(wg_hbm, wg_v, 2), cp(wu_hbm, wu_v, 2), cp(wd_hbm, wd_v, 2)]

    def start(g):
        for c in g:
            c.start()

    def wait(g):
        for c in g:
            c.wait()

    rk = [None] * 7
    lxs = {}

    def lx(t, i):
        if (t, i) not in lxs:
            lxs[t, i] = _operand(_LT[i], lambda q: x_v[q // 2, _TILES[t]:_TILES[t + 1], (q % 2) * HD:(q % 2 + 1) * HD])
        return lxs[t, i]

    def acc(ref, idx, v, op, first):
        ref[idx] = v if first else op(v, ref[idx])

    def kprod(t, i):
        n = _TILES[t + 1] - _TILES[t]
        v = _dot_nt(rk[i], lx(t, i))
        if i == 0:
            acc(ks_v, 0, _lanefold(jnp.abs(v), jnp.maximum), jnp.maximum, t == 0)

        def put(k, u):
            mo_v[k, 0:HD, 0:n] = u

        def fin(q, c):
            if q in (0, 3):
                acc(ks_v, 1 + q // 3, _lanefold(jnp.abs(c), jnp.add), jnp.add, t == 0)
            p = _phi(c)
            h_v[t % 4, (0, 2, 1, 3)[q], 0:HD, 0:n] = p
            acc(z_acc, (slice((q % 2) * HD, (q % 2 + 1) * HD),), _lanefold(p, jnp.add), jnp.add, t == 0 and q in (1, 2))

        _strassen_step(i, v, lambda k: mo_v[k, 0:HD, 0:n], put, fin)

    def pprod(t, i):
        n = _TILES[t + 1] - _TILES[t]
        l = _term(_LT[i], lambda q: h_v[t % 4, q, 0:HD, 0:n]).astype(BF)
        acc(p_acc, i, _dot(l, lx(t, _R_AS_L[i])), jnp.add, t == 0)

    start(g1)
    start(g2)
    start(g3)
    wait(g1)
    start(g4)
    ta = wqkv_v[:HD, D:2 * D].astype(F32).T
    rk[1] = ta[:HD].astype(BF)
    rk[5] = (ta[:HD] + ta[HD:]).astype(BF)
    wait(g2)
    start(g5)
    tb = wqkv_v[HD:, D:2 * D].astype(F32).T
    rk[0] = (ta[:HD] + tb[HD:]).astype(BF)
    rk[2] = (ta[HD:] - tb[HD:]).astype(BF)
    rk[3] = (tb[:HD] - ta[:HD]).astype(BF)
    rk[4] = tb[HD:].astype(BF)
    rk[6] = (tb[:HD] + tb[HD:]).astype(BF)
    wait(g3)
    start(g6)
    for i in _ORD:
        kprod(0, i)
    for i in _P_ORD[:5]:
        pprod(0, i)
    wait(g4)
    for i in _P_ORD[5:]:
        pprod(0, i)
    for i in _ORD:
        kprod(1, i)
    for i, j in zip(_ORD, _P_ORD):
        kprod(2, i)
        pprod(1, j)
    for i in _P_ORD[:6]:
        pprod(2, i)
    wait(g5)
    pprod(2, _P_ORD[6])
    gf_v[...] = jnp.broadcast_to(gw_v[...].astype(F32).reshape(1, D), (8, D))
    blocks = _perm_lanes([pltpu.bitcast(wqkv_v[:, j * L:(j + 1) * L], jnp.uint32) for j in range(4)])
    for j in range(4):
        wq_v[0:HD, j * L:(j + 1) * L] = blocks[j]
    for i in _ORD:
        kprod(3, i)
    p_jobs = [(t, i) for t in (3, 4) for i in _P_ORD]
    for i in _ORD:
        kprod(4, i)
        if i in _P_IN_K:
            pprod(*p_jobs.pop(0))

    zrow = jnp.sum(z_acc[...].T, axis=0, keepdims=True)
    zb = _perm_lanes([jnp.broadcast_to(zrow[:, j * L:(j + 1) * L], (8, L)) for j in range(4)])
    zr = jnp.concatenate(zb, axis=1)[0:1, :]
    rqs = {}
    qs = {}
    q_growth = []

    def rq(i):
        if i not in rqs:
            rqs[i] = _operand(_RT[i], lambda q: pltpu.bitcast(
                wq_v[(q // 2) * L:(q // 2 + 1) * L, (q % 2) * HD:(q % 2 + 1) * HD], BF))
        return rqs[i]

    def gate(k, rows):
        gl = jnp.sum(x_v[k, rows, :].astype(F32) * gf_v[...][0:1, :], axis=1, keepdims=True)
        th = jnp.broadcast_to(jnp.tanh(0.5 * gl), (rows.stop - rows.start, L))
        hs = 0.25 - 0.25 * th
        g_v[k, rows, :] = hs
        if rows.start < HM:
            h_v[4, k, rows, 0:L] = hs
        return 0.5 + 0.5 * th

    def qprod(t, i):
        rows = slice(_TILES[t], _TILES[t + 1])
        n = _TILES[t + 1] - _TILES[t]
        v = _dot(lx(t, i), rq(i))
        if i == 0:
            qs["g"] = _colmax(v)
        if i in _GATE_AT:
            gf_v[1:2, :] = jnp.concatenate([v[0:1, :], v[0:1, :]], axis=1)
            qs["gate", _GATE_AT.index(i)] = gate(_GATE_AT.index(i), rows)

        def put(k, u):
            mo_v[k, HD:HD + n, :] = u

        def fin(q, c):
            k, cols = q // 2, slice((q % 2) * HD, (q % 2 + 1) * HD)
            if q in (0, 3):
                qs[q] = _colsum(c[:L])
                if q == 3:
                    q_growth.append(qs["g"] - (KAPPA / L) * jnp.minimum(qs[0], qs[3]))
            pq = _phi(c)
            s = _lanefold(pq * zr[:, cols], jnp.add)
            if q in (1, 2):
                pq_v[k, rows, cols] = pq
                mo_v[4 + k, 0:n, 0:L] = s
                return
            s = s + mo_v[4 + k, 0:n, 0:L]
            lane = lax.broadcasted_iota(jnp.int32, (n, L), 1)
            s = s + jnp.where((lane & 1) == 0, pltpu.roll(s, L - 1, 1), pltpu.roll(s, 1, 1))
            s = s + jnp.where((lane & 2) == 0, pltpu.roll(s, L - 2, 1), pltpu.roll(s, 2, 1))
            den = s + 1e-6
            inv = pl.reciprocal(den, approx=True)
            inv = inv * (2.0 - den * inv)
            scale = qs["gate", k] * inv
            scale = jnp.concatenate([scale, scale], axis=1)
            other = slice(HD - cols.start, 2 * HD - cols.start)
            pq_v[k, rows, cols] = pq * scale
            pq_v[k, rows, other] = pq_v[k, rows, other] * scale

        _strassen_step(i, v, lambda k: mo_v[k, HD:HD + n, :], put, fin)

    pprod(*p_jobs.pop(0))
    for t in _Q_TILES:
        for i in _ORD:
            qprod(t, i)
            if i in _P_IN_Q and p_jobs:
                pprod(*p_jobs.pop(0))
    assert not p_jobs

    same = (lax.broadcasted_iota(jnp.int32, (L, L), 0) // DH) == (lax.broadcasted_iota(jnp.int32, (L, L), 1) // DH)
    kvs = []
    pdiag = []
    for b in range(D // L):
        rs = slice((b % 2) * L, (b % 2 + 1) * L)
        pb = [_term(_CT[2 * (b // 2) + c], lambda j: p_acc[j, rs, :]) for c in range(2)]
        pdiag.append(pb[b // 2])
        kv = _dot(jnp.concatenate(pb, axis=1).astype(BF), wqkv_v[:, 2 * D + b * L: 2 * D + (b + 1) * L])
        kvs.append(jnp.where(same, kv, 0.0).astype(BF))
    p11, p22 = jnp.concatenate(pdiag[:2], axis=0), jnp.concatenate(pdiag[2:], axis=0)
    sub_lo = lax.broadcasted_iota(jnp.int32, (16, 8, HD), 1) < 4
    for b1 in range(2):
        for c in range(2):
            cols = slice(c * HD, (c + 1) * HD)
            u, v = [_dot(kvs[b], wo_v[b * L:(b + 1) * L, cols]).reshape(16, 8, HD) for b in (2 * b1, 2 * b1 + 1)]
            for d2, w in enumerate((jnp.where(sub_lo, u, pltpu.roll(v, 4, 1)), jnp.where(sub_lo, pltpu.roll(u, 4, 1), v))):
                for e in range(16):
                    r = (2 * (e % 2) + d2) * L + (e // 2) * 16 + b1 * 8
                    m_v[r:r + 8, cols] = w[e]

    pm = p_acc[0]
    chk_v[0:1, :] = functools.reduce(jnp.maximum, q_growth)
    chk_v[1:2, :] = _colmax(pm) - (KAPPA / HD) * jnp.minimum(_colsum(p11), _colsum(p22))
    stats = ((_lanefold(jnp.abs(pm), jnp.maximum), _lanefold(jnp.abs(p11), jnp.add), _lanefold(jnp.abs(p22), jnp.add), HD),
             (ks_v[0], ks_v[1], ks_v[2], HS))
    for r, (kg, k1, k2, n) in enumerate(stats):
        kt = jnp.minimum(jnp.sum(k1, axis=1, keepdims=True), jnp.sum(k2, axis=1, keepdims=True))
        km = jnp.max(kg - (KAPPA / n) * kt, axis=0, keepdims=True)
        chk_v[2 + r:3 + r, :] = jnp.concatenate([km, km], axis=1)
    chk_v[4:8, :] = jnp.zeros((4, HD), F32)

    wait(g6)

    def ffn(t, carry):
        r0 = pl.multiple_of(t * HM, HM)

        h_v[5, t, 0:8, 0:L] = jnp.zeros((8, L), F32)
        acc_v[49 + t, 0:8, :] = jnp.zeros((8, L), F32)
        mo_v[7 + t, 0:8, 0:L] = jnp.zeros((8, L), F32)
        p_acc[7 + t, 0:8, 0:L] = jnp.zeros((8, L), F32)
        gf_v[pl.ds(2 + t, 1), :] = jnp.zeros((1, D), F32)
        wq_v[pl.ds(pl.multiple_of(HD + 8 * t, 8), 8), 0:L] = jnp.zeros((8, L), jnp.uint32)
        go_v[7 + t, 0, 0, 0:8, :] = jnp.zeros((8, L), F32)
        rt_v[2 + t, 0, 0, 0:8, :] = jnp.zeros((8, L), F32)

        seen = set()
        singles = []
        sets = []

        def queue(getl, getr, outers, whole, order):
            for i in outers:
                if i in whole:
                    sets.append((i, _SET_A, getl, getr))
                    sets.append((i, _SET_B, getl, getr))
                else:
                    for j in order:
                        singles.append((i, j, getl, getr))

        def put_leaf(i, j, p):
            k = 7 * i + j
            acc_v[k] = p + acc_v[k] if k in seen else p
            seen.add(k)

        def single(n):
            for _ in range(min(n, len(singles))):
                i, j, getl, getr = singles.pop(0)
                put_leaf(i, j, _dot(_term(_leaf_terms(_LT, i, j), getl).astype(BF),
                                    _term(_leaf_terms(_RT, i, j), getr).astype(BF)))

        def issue(n):
            if n % 4:
                single(n)
                return
            for _ in range(n // 4):
                if not sets:
                    single(4)
                    continue
                i, js, getl, getr = sets.pop(0)
                lo = [_term(_LT[i], lambda q1: getl((q1, q2))) for q2 in range(4)]
                ro = [_term(_RT[i], lambda q1: getr((q1, q2))) for q2 in range(4)]
                for j in js:
                    put_leaf(i, j, _dot(_term(_LT[j], lambda q: lo[q]).astype(BF), _term(_RT[j], lambda q: ro[q]).astype(BF)))
                single(4 - len(js))

        def geth(g, q):
            q1, q2 = q
            return h_v[g, q1, (q2 // 2) * QM:(q2 // 2 + 1) * QM, (q2 % 2) * L:(q2 % 2 + 1) * L]

        def getwd(g, q):
            q1, q2 = q
            r = (2 * g + q2 // 2) * FC + (q1 // 2) * L
            c = (q1 % 2) * HD + (q2 % 2) * L
            return wd_v[r:r + L, c:c + L].astype(F32)

        def getq(q):
            q1, q2 = q
            c = (q1 % 2) * HD + (q2 % 2) * L
            return pq_v[q1 // 2, (q2 // 2) * QM:(q2 // 2 + 1) * QM, c:c + L]

        def getm(q):
            q1, q2 = q
            r = (q1 // 2) * HD + (q2 // 2) * L
            c = (q1 % 2) * HD + (q2 % 2) * L
            return m_v[r:r + L, c:c + L]

        queue(getq, getm, *_DOWN[0])
        singles.sort(key=lambda e: not (e[0] in (1, 4) and e[1] in (1, 4)))
        single(4)

        l2 = {}
        growth = []

        def xblk(q1, q2):
            c = (q1 % 2) * HD + (q2 % 2) * L
            return x_v[q1 // 2, pl.ds(pl.multiple_of(r0 + (q2 // 2) * QM, QM), QM), c:c + L]

        def gate_up(g):
            half = g == NCH // 2
            mats = (0,) if half else (1, 0)
            gmax = {}
            tmin = {}

            def wblk(w, q1, q2):
                r = (q1 // 2) * HD + (q2 // 2) * L
                c = (2 * g + (0 if half else q2 % 2)) * FC + (q1 % 2) * L
                return (wg_v, wu_v)[q2 % 2 if half else w][r:r + L, c:c + L]

            def fin(w, q2, q1, c):
                if q1 in (0, 3) and q2 in (0, 3):
                    v = _colsum(c.reshape(QM // 16, 2, 8, L)[:, 0].reshape(QM // 2, L))
                    tmin[w] = jnp.minimum(tmin[w], v) if w in tmin else v
                c2 = 0 if half else q2 % 2
                dst = (g, q1, slice((q2 // 2) * QM, (q2 // 2 + 1) * QM), slice(c2 * L, (c2 + 1) * L))
                first = q2 in (1, 2) if half else w == 1
                is_gate = q2 % 2 == 0 if half else w == 0
                o = h_v[4, q1 // 2, (q2 // 2) * QM:(q2 // 2 + 1) * QM, 0:L] if first else h_v[dst]
                h_v[dst] = (c * o) * (1.0 + jnp.tanh(0.5 * c)) if is_gate else c * o

            for n, i in enumerate(_ORD):
                shared = len(_RT[i]) > 1
                if shared:
                    for w in mats:
                        for q2 in range(4):
                            rt_v[n % 2, w, q2] = _term(_RT[i], lambda q1: wblk(w, q1, q2).astype(F32))

                def leaves(w, js):
                    if (i, js[0]) not in l2:
                        xq = [_term(_LT[i], lambda q1: xblk(q1, q2).astype(F32)) for q2 in range(4)]
                        for j in js:
                            terms = _leaf_terms(_LT, i, j)
                            l2[i, j] = xblk(*terms[0][1]) if len(terms) == 1 else _term(_LT[j], lambda q2: xq[q2]).astype(BF)
                    out = []
                    for j in js:
                        if shared:
                            r = _term(_RT[j], lambda q2: rt_v[n % 2, w, q2]).astype(BF)
                        else:
                            r = _operand(_RT[j], lambda q2: wblk(w, _RT[i][0][1], q2))
                        out.append(_dot(l2[i, j], r))
                    return out

                def done(w, q2, v):
                    def put(k, u):
                        go_v[k, w, q2] = u

                    _strassen_step(i, v, lambda k: go_v[k, w, q2], put, functools.partial(fin, w, q2))

                for w in mats:
                    m3, m5, m2, m4 = leaves(w, _SET_A)
                    go_v[4, w, 0] = m4 - m5
                    go_v[4, w, 3] = m3 - m2
                    done(w, 1, m3 + m5)
                    done(w, 2, m2 + m4)
                    m1, m7, m6 = leaves(w, _SET_B)
                    issue(1)
                    for v in {0: (m1, m7, m6), 5: (m1,), 6: (m1,)}.get(i, ()):
                        v = _colmax(v)
                        gmax[w] = jnp.maximum(gmax[w], v) if w in gmax else v
                    done(w, 0, (m1 + m7) + go_v[4, w, 0])
                    done(w, 3, (m1 + m6) + go_v[4, w, 3])
                issue(_EXTRA[g][n])
            gm = jnp.concatenate([gmax[0], gmax[mats[0]]], axis=1)
            tm = jnp.concatenate([tmin[0], tmin[mats[0]]], axis=1)
            growth.append(gm - (KAPPA2 / (QM // 2)) * tm)

        for g in range(NCH // 2 + 1):
            gate_up(g)
            if g < NCH // 2:
                queue(functools.partial(geth, g), functools.partial(getwd, g), *_DOWN[g + 1])
        assert not singles and not sets
        pq_v[:, 0:HM, :] = pq_v[:, HM:2 * HM, :]
        for k in range(2):
            h_v[4, k, :, 0:L] = g_v[k, HM:2 * HM, :]

        def rest(i, chunks, ks=slice(None)):
            ls = [_term(_LT[i], lambda q: h_v[c // 2, q, ks, (c % 2) * L:(c % 2 + 1) * L]) for c in chunks]
            rs = [_term(_RT[i], lambda q: wd_v[c * FC + (q // 2) * L:c * FC + (q // 2 + 1) * L,
                                               (q % 2) * HD:(q % 2 + 1) * HD].astype(F32)) for c in chunks]
            return _dot(jnp.concatenate(ls, axis=1).astype(BF), jnp.concatenate(rs, axis=0).astype(BF))

        def outer(i, chunks=None, k0=0, nr=HM):
            if chunks is None:
                chunks = [NCH - 1] if i in _DOWN[3][0] else [NCH - 3, NCH - 2, NCH - 1]
            v = rest(i, chunks, slice(k0, k0 + nr))
            n = min(nr, QM)
            out = []
            for a in range(k0, k0 + nr, n):
                cols = []
                for c2 in range(2):
                    u = v[a - k0:a - k0 + n, c2 * L:(c2 + 1) * L]
                    for sg, j in _CT[2 * (a // QM) + c2]:
                        p = acc_v[7 * i + j, a % QM:a % QM + n, :]
                        u = u + p if sg > 0 else u - p
                    cols.append(u)
                out.append(jnp.concatenate(cols, axis=1))
            return jnp.concatenate(out, axis=0)

        def emit(k, k0, c0, val):
            nr, nc = val.shape
            rows = pl.ds(pl.multiple_of(r0 + k0, nr), nr)
            o_buf[k, rows, c0:c0 + nc] = val.astype(BF)
            cp(o_buf.at[k, rows, pl.ds(c0, nc)], out_hbm.at[k, rows, pl.ds(c0, nc)], 0).start()

        mo_v[3] = outer(3, [NCH - 3, NCH - 2])
        mo_v[2] = outer(2)
        m5 = outer(4)
        mo_v[4] = m5
        emit(0, 0, HD, m5 + mo_v[2])
        mo_v[1] = outer(1)
        m4 = rest(3, [NCH - 1]) + mo_v[3]
        mo_v[3] = m4 - mo_v[4]
        emit(1, 0, 0, m4 + mo_v[1])
        m1 = outer(0)
        mo_v[3] = m1 + mo_v[3]
        mo_v[5] = (m1 - mo_v[1]) + mo_v[2]
        for k0 in range(0, HM, QM):
            o11 = outer(6, None, k0, QM) + mo_v[3, k0:k0 + QM, :]
            emit(0, k0, 0, o11)
        gl = functools.reduce(jnp.maximum, [_colmax(acc_v[7 * i]) for i in (0, 5, 6)])
        chk_v[4:5, :] = jnp.maximum(chk_v[4:5, :], functools.reduce(jnp.maximum, growth))
        chk_v[5:6, :] = jnp.maximum(chk_v[5:6, :], jnp.maximum(_colmax(m1), jnp.concatenate([gl, gl], axis=1)))
        chk_v[6:7, :] = jnp.maximum(chk_v[6:7, :], _colmax(o11))
        for k0, nr, piece in ((0, QM, QM), (QM, L, L), (QM + L, L, L // 2)):
            res = outer(5, None, k0, nr) + mo_v[5, k0:k0 + nr, :]
            for e in range(0, nr, piece):
                emit(1, k0 + e, HD, res[e:e + piece])
        return carry

    lax.fori_loop(0, HS // HM, ffn, 0)
    omax = jnp.max(chk_v[6:7, :])
    ok = jnp.logical_and(jnp.max(chk_v[0:5, :]) <= 0.0, jnp.max(chk_v[5:6, :]) <= KAPPA_OUT * omax)
    cp(o_buf, out_hbm, 0).wait()

    @pl.when(jnp.logical_not(ok))
    def _classical():
        nt = HS // L

        def tile(i):
            return i // nt, pl.ds(pl.multiple_of((i % nt) * L, L), L)

        def blk(b, base=0):
            return pl.ds(pl.multiple_of(base + b * L, L), L)

        def head_block(b, carry):
            fa_v[blk(b), :] = wqkv_v[:, blk(b, D)].astype(F32).T.astype(BF)
            m_v[0:L, :] = jnp.zeros((L, D), F32)

            def kbody(i, z):
                k, rows = tile(i)
                xt = x_v[k, rows, :]
                pkt = _phi(_dot_nt(fa_v[blk(b), :], xt))
                m_v[0:L, :] += _dot(pkt.astype(BF), xt)
                return z + pkt

            z = lax.fori_loop(0, 2 * nt, kbody, jnp.zeros((L, L), F32))
            kv = jnp.where(same, _dot(m_v[0:L, :].astype(BF), wqkv_v[:, blk(b, 2 * D)]), 0.0).astype(BF)
            fa_v[blk(b), :] = _dot(kv, wo_v[blk(b), :]).astype(BF)
            z = jnp.broadcast_to(jnp.sum(z, axis=1, keepdims=True), (L, L))
            fz_v[b] = jnp.where(same, z, 0.0).astype(BF)
            return carry

        lax.fori_loop(0, D // L, head_block, 0)

        def obody(i, carry):
            k, rows = tile(i)
            m_v[0:L, :] = jnp.zeros((L, D), F32)

            def abody(b, c):
                pq = _phi(_dot(x_v[k, rows, :], wqkv_v[:, blk(b)]))
                den = _dot(pq.astype(BF), fz_v[b]) + 1e-6
                m_v[0:L, :] += _dot((pq * ((1.0 - 2.0 * g_v[k, rows, :]) / den)).astype(BF), fa_v[blk(b), :])
                return c

            def fbody(f, c):
                xt = x_v[k, rows, :]
                g = _dot(xt, wg_v[:, blk(f)])
                h = (g * g_v[k, rows, :]) * (1.0 + jnp.tanh(0.5 * g)) * _dot(xt, wu_v[:, blk(f)])
                m_v[0:L, :] += _dot(h.astype(BF), wd_v[blk(f), :])
                return c

            lax.fori_loop(0, D // L, abody, 0)
            lax.fori_loop(0, F // L, fbody, 0)
            o_buf[k, rows, :] = m_v[0:L, :].astype(BF)
            return carry

        lax.fori_loop(0, 2 * nt, obody, 0)
        cp(o_buf, out_hbm, 0).start()
        cp(o_buf, out_hbm, 0).wait()

    return omax < 0.0


def _kernel(*refs):
    lax.while_loop(lambda again: again, lambda _: _body(*refs), jnp.bool_(True))


@jax.jit
def pallas_gated_mix__linear_attn_block__swiglu_ffn__prompt_kernel(
    A_x: jax.Array,
    A_wqkv: jax.Array,
    A_wo: jax.Array,
    B_x: jax.Array,
    B_w_gate: jax.Array,
    B_w_up: jax.Array,
    B_w_down: jax.Array,
    gate_w: jax.Array,
):
    del B_x
    hbm = pl.BlockSpec(memory_space=pl.ANY)
    out = pl.pallas_call(
        _kernel,
        out_shape=jax.ShapeDtypeStruct((2, HS, D), BF),
        in_specs=[hbm] * 7,
        out_specs=hbm,
        scratch_shapes=[
            pltpu.VMEM((2, HS, D), BF),
            pltpu.VMEM((D, 3 * D), BF),
            pltpu.VMEM((D, D), BF),
            pltpu.VMEM((D, F), BF),
            pltpu.VMEM((D, F), BF),
            pltpu.VMEM((F, D), BF),
            pltpu.VMEM((D,), BF),
            pltpu.VMEM((8, D), F32),
            pltpu.VMEM((HD + 16, D), jnp.uint32),
            pltpu.VMEM((9, 2, 4, QM, L), F32),
            pltpu.VMEM((4, 2, 4, L, L), F32),
            pltpu.VMEM((9, HD, HD), F32),
            pltpu.VMEM((D, L), F32),
            pltpu.VMEM((D, D), F32),
            pltpu.VMEM((6, 4, HM, HD), F32),
            pltpu.VMEM((51, QM, L), F32),
            pltpu.VMEM((9, HM, HD), F32),
            pltpu.VMEM((2, HS, D), F32),
            pltpu.VMEM((2, HS, L), F32),
            pltpu.VMEM((3, HD, L), F32),
            pltpu.VMEM((8, HD), F32),
            pltpu.VMEM((D, D), BF),
            pltpu.VMEM((D // L, L, L), BF),
            pltpu.VMEM((2, HS, D), BF),
            pltpu.SemaphoreType.DMA((3,)),
        ],
        compiler_params=pltpu.CompilerParams(
            vmem_limit_bytes=100 * 1024 * 1024,
            disable_bounds_checks=True,
            disable_semaphore_checks=True,
        ),
    )(A_x.reshape(2, HS, D), A_wqkv, A_wo, B_w_gate, B_w_up, B_w_down, gate_w)
    return out.reshape(1, S, D)
```
